```python
import jax
import jax.numpy as jnp

def _softmax(x, axis=-1):
    return jax.nn.softmax(x, axis=axis)

def _gelu(x):
    return jax.nn.gelu(x, approximate=True)

def _silu(x):
    return jax.nn.silu(x)

def _sigmoid(x):
    return jax.nn.sigmoid(x)

def _layernorm(x, axis=-1, eps=1e-05):
    m = jnp.mean(x, axis=axis, keepdims=True)
    v = jnp.var(x, axis=axis, keepdims=True)
    return (x - m) / jnp.sqrt(v + eps)

def _scatter_add(tgt, idx, src, axis=0):
    return tgt.at[idx].add(src)

def _segment_sum(src, seg, n):
    return jax.ops.segment_sum(src, seg, n)

class _Rng:

    def __init__(self, key):
        self._k = key

    def _next(self):
        self._k, sub = jax.random.split(self._k)
        return sub

    def normal(self, shape):
        return jax.random.normal(self._next(), shape, dtype=jnp.bfloat16)

    def randint(self, lo, hi, shape):
        return jax.random.randint(self._next(), shape, lo, hi, dtype=jnp.int32)

    def uniform(self, shape, lo=0.0, hi=1.0):
        return jax.random.uniform(self._next(), shape, jnp.bfloat16, lo, hi)

    def permutation(self, n):
        return jax.random.permutation(self._next(), n)
kernel_name = 'interleave_layers__memory_aug_recurrent_mem_tr__sliding_local_dilated__prompt'

def setup_inputs():
    _rng = _Rng(jax.random.key(int.from_bytes(__import__("os").urandom(4), "little")))
    _w = lambda a: (lambda t: t.astype(jnp.bfloat16) if jnp.issubdtype(t.dtype, jnp.floating) else t)(jnp.asarray(a))

    def _A_setup():
        B, S, Dm = (1, 2048, 640)
        H, Dh = (32, 192)
        M, seg = (8, 32)
        seg = min(seg, S)
        S = S // seg * seg
        return {'x': _w((lambda *s: _rng.normal(s) * 0.05)(B, S, Dm)), 'mem0': _w((lambda *s: _rng.normal(s) * 0.05)(B, M, Dm)), 'Wq': _w((lambda *s: _rng.normal(s) * 0.05)(Dm, H, Dh) * Dm ** (-0.5)), 'Wk': _w((lambda *s: _rng.normal(s) * 0.05)(Dm, H, Dh) * Dm ** (-0.5)), 'Wv': _w((lambda *s: _rng.normal(s) * 0.05)(Dm, H, Dh) * Dm ** (-0.5)), 'Wo': _w((lambda *s: _rng.normal(s) * 0.05)(H, Dh, Dm) * (H * Dh) ** (-0.5)), 'seg_len': seg}
    _A_in = _A_setup()

    def _B_setup():
        B, S, D = (1, 2048, 640)
        return {'x': _w((lambda *s: _rng.normal(s) * 0.05)(B, S, D)), 'wqkv': _w((lambda *s: _rng.normal(s) * 0.05)(D, 3 * D)), 'wo': _w((lambda *s: _rng.normal(s) * 0.05)(D, D))}
    _B_in = _B_setup()
    return {'A_x': _A_in['x'], 'A_mem0': _A_in['mem0'], 'A_Wq': _A_in['Wq'], 'A_Wk': _A_in['Wk'], 'A_Wv': _A_in['Wv'], 'A_Wo': _A_in['Wo'], 'A_seg_len': _A_in['seg_len'], 'B_x': _B_in['x'], 'B_wqkv': _B_in['wqkv'], 'B_wo': _B_in['wo']}

def reference(A_x, A_mem0, A_Wq, A_Wk, A_Wv, A_Wo, A_seg_len, B_x, B_wqkv, B_wo):

    def _A_ref(x, mem0, Wq, Wk, Wv, Wo, seg_len):
        B, S, Dm = x.shape
        H, Dh = (Wq.shape[1], Wq.shape[2])
        M = mem0.shape[1]
        scale = Dh ** (-0.5)
        n_seg = S // seg_len
        L = M + seg_len
        idx = jnp.arange(L)
        mask = (idx[:, None] < M) | (idx[:, None] >= idx[None, :])
        mem = mem0
        outs = []
        for s in range(n_seg):
            xs = x[:, s * seg_len:(s + 1) * seg_len, :].copy()
            h = jnp.concatenate([mem, xs], axis=1)
            q = jnp.einsum('btd,dhe->bhte', h, Wq)
            k = jnp.einsum('btd,dhe->bhte', h, Wk)
            v = jnp.einsum('btd,dhe->bhte', h, Wv)
            scores = jnp.einsum('bhqe,bhke->bhqk', q, k) * scale
            scores = jnp.where(mask[None, None], scores, -1000000000.0)
            p = _softmax(scores, axis=-1)
            o = jnp.einsum('bhqk,bhke->bhqe', p, v)
            o = jnp.einsum('bhte,hed->btd', o, Wo)
            mem = o[:, :M, :].copy()
            outs.append(o[:, M:, :])
        return jnp.concatenate(outs, axis=1)

    def _B_ref(x, wqkv, wo):
        B, S, D = x.shape
        H = 32
        Dh = D // H
        W, dil = (8, 2)
        qkv = (lambda x, *d: x.transpose(*d))((x @ wqkv).reshape(B, S, 3, H, Dh), 2, 0, 3, 1, 4)
        q, k, v = (qkv[0], qkv[1], qkv[2])
        scale = Dh ** (-0.5)
        pos = jnp.arange(S)
        off = jnp.arange(W) * dil
        idx = pos[:, None] - off[None, :]
        mask = idx >= 0
        idx_c = jnp.where(mask, idx, 0).reshape(-1)
        kg = k[:, :, idx_c, :].reshape(B, H, S, W, Dh)
        vg = v[:, :, idx_c, :].reshape(B, H, S, W, Dh)
        logits = jnp.einsum('bhsd,bhswd->bhsw', q, kg) * scale
        logits = jnp.where(mask[None, None, :, :], logits, -1000000000.0)
        attn = _softmax(logits, axis=-1)
        o = jnp.einsum('bhsw,bhswd->bhsd', attn, vg)
        return (lambda x, *d: x.transpose(*d))(o, 0, 2, 1, 3).reshape(B, S, D) @ wo
    x = A_x
    x = x + _A_ref(_layernorm(x, axis=-1), A_mem0, A_Wq, A_Wk, A_Wv, A_Wo, A_seg_len)
    x = x + _B_ref(_layernorm(x, axis=-1), B_wqkv, B_wo)
    x = x + _A_ref(_layernorm(x, axis=-1), A_mem0, A_Wq, A_Wk, A_Wv, A_Wo, A_seg_len)
    x = x + _B_ref(_layernorm(x, axis=-1), B_wqkv, B_wo)
    return x
```

```python
import functools

import jax
import jax.numpy as jnp
from jax import lax
import jax.experimental.pallas as pl
import jax.experimental.pallas.tpu as pltpu

F32 = jnp.float32
BF16 = jnp.bfloat16
NT = (((1,), (1,)), ((), ()))
NN = (((1,), (0,)), ((), ()))


def _ln(x):
    m = jnp.mean(x, axis=-1, keepdims=True)
    xc = x - m
    v = jnp.mean(xc * xc, axis=-1, keepdims=True)
    return xc * lax.rsqrt(v + 1e-5)


def _dot(a, b, dims=NN):
    return lax.dot_general(a, b, dims, preferred_element_type=F32)


def _kernel(x_ref, mem0_ref, wq_ref, wk_ref, wv_ref, wo_ref, bqkv_ref, bwo_ref,
            out_ref,
            h_ref, y_ref, x2_ref, kb_ref, vb_ref, bqkvp_ref, bwop_ref,
            *, S, D, H, DH, M, SEG, HB, W, DIL):
    NSEG = S // SEG
    NP = H // 2
    PW = 2 * DH
    scale_a = DH ** -0.5
    DHB = D // HB
    scale_b = DHB ** -0.5

    ri = lax.broadcasted_iota(jnp.int32, (D, D), 0)
    ci = lax.broadcasted_iota(jnp.int32, (D, D), 1)
    pm = (ri == (ci % HB) * DHB + ci // HB).astype(BF16)
    pmt = (ci == (ri % HB) * DHB + ri // HB).astype(BF16)
    for j in range(3):
        bqkvp_ref[:, j * D:(j + 1) * D] = _dot(bqkv_ref[:, j * D:(j + 1) * D], pm).astype(BF16)
    bwop_ref[...] = _dot(pmt, bwo_ref[...]).astype(BF16)

    mem0 = mem0_ref[...].astype(F32)
    h_ref[0:16, :] = jnp.concatenate([mem0, mem0], axis=0).astype(BF16)
    h_ref[16:48, :] = _ln(x_ref[0:SEG, :].astype(F32)).astype(BF16)
    h_ref[48:80, :] = jnp.zeros((SEG, D), BF16)
    y_ref[...] = jnp.zeros(y_ref.shape, F32)
    x2_ref[...] = jnp.zeros(x2_ref.shape, F32)
    kb_ref[...] = jnp.zeros(kb_ref.shape, F32)
    vb_ref[...] = jnp.zeros(vb_ref.shape, F32)

    r = lax.broadcasted_iota(jnp.int32, (48, 128), 0)
    l = lax.broadcasted_iota(jnp.int32, (48, 128), 1)
    slot = jnp.where(l >= 48, l - 48, l)
    xvalid = (slot >= 16) & ((r < 16) | (r >= slot)) & (l < 96)
    valid = [xvalid | ((slot < 8) & (l < 96)), xvalid | ((slot >= 8) & (slot < 16) & (l < 96))]
    lane_h = l < 48
    lane128 = lax.broadcasted_iota(jnp.int32, (80, 128), 1)
    lo = lane128 < 64

    def rows_c(a, c):
        return jnp.concatenate([a[0:16], a[16 + 32 * c:48 + 32 * c]], axis=0)

    def blk(a, c):
        a0, a1, a2 = a[:, 0:128], a[:, 128:256], a[:, 256:384]
        a1h = jnp.where(lo, a1, 0.0)
        a1g = jnp.where(lo, 0.0, a1)
        z = jnp.zeros((48, 128), BF16)
        top = jnp.concatenate([rows_c(a0, c).astype(BF16), rows_c(a1h, c).astype(BF16), z], axis=1)
        mid = jnp.concatenate([z, rows_c(a1g, c).astype(BF16), rows_c(a2, c).astype(BF16)], axis=1)
        return jnp.concatenate([top, mid, jnp.zeros((32, PW), BF16)], axis=0)

    def a_step(h):
        acc = None
        for p in range(NP):
            q = _dot(h, wq_ref[p * PW:(p + 1) * PW, :], NT)
            k = _dot(h, wk_ref[p * PW:(p + 1) * PW, :], NT)
            v = _dot(h, wv_ref[p * PW:(p + 1) * PW, :], NT)
            os_ = []
            for c in range(2):
                qc = rows_c(q, c).astype(BF16)
                s = _dot(qc, blk(k, c), NT) * scale_a
                s = jnp.where(valid[c], s, -1e9)
                mh = jnp.max(jnp.where(lane_h, s, -jnp.inf), axis=-1, keepdims=True)
                mg = jnp.max(jnp.where(lane_h, -jnp.inf, s), axis=-1, keepdims=True)
                e = jnp.exp(s - jnp.where(lane_h, mh, mg))
                lh = jnp.sum(jnp.where(lane_h, e, 0.0), axis=-1, keepdims=True)
                lg = jnp.sum(jnp.where(lane_h, 0.0, e), axis=-1, keepdims=True)
                pr = (e * jnp.where(lane_h, 1.0 / lh, 1.0 / lg)).astype(BF16)
                os_.append(_dot(pr, blk(v, c)))
            o = jnp.concatenate([os_[0][0:8], os_[1][8:16], os_[0][16:48], os_[1][16:48]], axis=0).astype(BF16)
            d = _dot(o, wo_ref[p * PW:(p + 1) * PW, :])
            acc = d if acc is None else acc + d
        return acc

    rowi = lax.broadcasted_iota(jnp.int32, (SEG, 128), 0)

    def b_block(t):
        y = y_ref[...]
        hb = _ln(y).astype(BF16)
        qkv = _dot(hb, bqkvp_ref[...])
        outs = []
        for lyr in range(2):
            seg = t - 1 - 2 * lyr
            q = qkv[32 * lyr:32 * lyr + 32, 0:D]
            kb_ref[lyr, 16:48, :] = qkv[32 * lyr:32 * lyr + 32, D:2 * D]
            vb_ref[lyr, 16:48, :] = qkv[32 * lyr:32 * lyr + 32, 2 * D:3 * D]
            logits = []
            for w in range(W):
                ks = kb_ref[lyr, 16 - DIL * w:48 - DIL * w, :]
                pr = q * ks
                tt = pr[:, 0:128] + pr[:, 128:256] + pr[:, 256:384] + pr[:, 384:512] + pr[:, 512:640]
                tt = tt + pltpu.roll(tt, 64, 1)
                tt = tt + pltpu.roll(tt, 32, 1)
                tt = tt * scale_b
                if w > 0:
                    tt = jnp.where(rowi + seg * SEG >= DIL * w, tt, -1e9)
                logits.append(tt)
            mx = functools.reduce(jnp.maximum, logits)
            es = [jnp.exp(t_ - mx) for t_ in logits]
            inv = 1.0 / functools.reduce(lambda a, b: a + b, es)
            o = None
            for w in range(W):
                a = es[w] * inv
                vs = vb_ref[lyr, 16 - DIL * w:48 - DIL * w, :]
                c = vs * jnp.concatenate([a] * 5, axis=1)
                o = c if o is None else o + c
            outs.append(o)
            kb_ref[lyr, 0:16, :] = kb_ref[lyr, 32:48, :]
            vb_ref[lyr, 0:16, :] = vb_ref[lyr, 32:48, :]
        o = jnp.concatenate(outs, axis=0).astype(BF16)
        return y + _dot(o, bwop_ref[...])

    def body(t, carry):
        h = h_ref[...]
        x2_res = x2_ref[...]
        z = b_block(t)
        x2_new = z[0:32]
        x2_ref[...] = x2_new
        h_ref[48:80, :] = _ln(x2_new).astype(BF16)

        @pl.when(t >= 3)
        def _():
            out_ref[pl.ds(pl.multiple_of((t - 3) * SEG, SEG), SEG), :] = z[32:64].astype(out_ref.dtype)

        tn = jnp.minimum(t + 1, NSEG - 1)
        h_ref[16:48, :] = _ln(x_ref[pl.ds(pl.multiple_of(tn * SEG, SEG), SEG), :].astype(F32)).astype(BF16)

        acc = a_step(h)
        m2 = jnp.where(t >= 2, acc[8:16], mem0)
        h_ref[0:16, :] = jnp.concatenate([acc[0:8], m2], axis=0).astype(BF16)
        tc = jnp.minimum(t, NSEG - 1)
        y_ref[0:32, :] = x_ref[pl.ds(pl.multiple_of(tc * SEG, SEG), SEG), :].astype(F32) + acc[16:48]
        y_ref[32:64, :] = x2_res + acc[48:80]
        return carry

    lax.fori_loop(0, NSEG + 2, body, 0)
    z = b_block(NSEG + 2)
    out_ref[pl.ds((NSEG - 1) * SEG, SEG), :] = z[32:64].astype(out_ref.dtype)


@functools.partial(jax.jit, static_argnames=("A_seg_len",))
def pallas_interleave_layers__memory_aug_recurrent_mem_tr__sliding_local_dilated__prompt_kernel(
    A_x: jax.Array,
    A_mem0: jax.Array,
    A_Wq: jax.Array,
    A_Wk: jax.Array,
    A_Wv: jax.Array,
    A_Wo: jax.Array,
    A_seg_len: int,
    B_x: jax.Array,
    B_wqkv: jax.Array,
    B_wo: jax.Array,
):
    del B_x
    B, S, D = A_x.shape
    _, H, DH = A_Wq.shape
    M = A_mem0.shape[1]
    SEG = int(A_seg_len)
    assert B == 1 and M == 8 and SEG == 32 and DH == 192 and D == 640

    x = A_x.reshape(S, D)
    mem0 = A_mem0.reshape(M, D)
    wq = A_Wq.transpose(1, 2, 0).reshape(H * DH, D)
    wk = A_Wk.transpose(1, 2, 0).reshape(H * DH, D)
    wv = A_Wv.transpose(1, 2, 0).reshape(H * DH, D)
    wo = A_Wo.reshape(H * DH, D)

    kern = functools.partial(_kernel, S=S, D=D, H=H, DH=DH, M=M, SEG=SEG, HB=32, W=8, DIL=2)
    out = pl.pallas_call(
        kern,
        out_shape=jax.ShapeDtypeStruct((S, D), A_x.dtype),
        scratch_shapes=[
            pltpu.VMEM((80, D), BF16),
            pltpu.VMEM((64, D), F32),
            pltpu.VMEM((SEG, D), F32),
            pltpu.VMEM((2, 48, D), F32),
            pltpu.VMEM((2, 48, D), F32),
            pltpu.VMEM((D, 3 * D), BF16),
            pltpu.VMEM((D, D), BF16),
        ],
        compiler_params=pltpu.CompilerParams(vmem_limit_bytes=110 * 1024 * 1024),
    )(x, mem0, wq, wk, wv, wo, B_wqkv, B_wo)
    return out.reshape(B, S, D)
```

```python
import functools

import jax
import jax.numpy as jnp
from jax import lax
import jax.experimental.pallas as pl
import jax.experimental.pallas.tpu as pltpu

F32 = jnp.float32
BF16 = jnp.bfloat16
NT = (((1,), (1,)), ((), ()))
NN = (((1,), (0,)), ((), ()))


def _ln(x):
    m = jnp.mean(x, axis=-1, keepdims=True)
    xc = x - m
    v = jnp.mean(xc * xc, axis=-1, keepdims=True)
    return xc * lax.rsqrt(v + 1e-5)


def _dot(a, b, dims=NN):
    return lax.dot_general(a, b, dims, preferred_element_type=F32)


def _kernel(x_ref, mem0_ref, wq_ref, wk_ref, wv_ref, wo_ref, bqkv_ref, bwo_ref,
            out_ref,
            h_ref, y_ref, x2_ref, kb_ref, vb_ref, bqkvp_ref, bwop_ref,
            *, S, D, H, DH, M, SEG, HB, W, DIL):
    NSEG = S // SEG
    NP = H // 2
    PW = 2 * DH
    scale_a = DH ** -0.5
    DHB = D // HB
    scale_b = DHB ** -0.5

    ri = lax.broadcasted_iota(jnp.int32, (D, D), 0)
    ci = lax.broadcasted_iota(jnp.int32, (D, D), 1)
    pm = (ri == (ci % HB) * DHB + ci // HB).astype(BF16)
    pmt = (ci == (ri % HB) * DHB + ri // HB).astype(BF16)
    for j in range(3):
        bqkvp_ref[:, j * D:(j + 1) * D] = _dot(bqkv_ref[:, j * D:(j + 1) * D], pm).astype(BF16)
    bwop_ref[...] = _dot(pmt, bwo_ref[...]).astype(BF16)

    mem0 = mem0_ref[...].astype(F32)
    h_ref[0:16, :] = jnp.concatenate([mem0, mem0], axis=0).astype(BF16)
    h_ref[16:48, :] = _ln(x_ref[0:SEG, :].astype(F32)).astype(BF16)
    h_ref[48:80, :] = jnp.zeros((SEG, D), BF16)
    y_ref[...] = jnp.zeros(y_ref.shape, F32)
    x2_ref[...] = jnp.zeros(x2_ref.shape, F32)
    kb_ref[...] = jnp.zeros(kb_ref.shape, F32)
    vb_ref[...] = jnp.zeros(vb_ref.shape, F32)

    r = lax.broadcasted_iota(jnp.int32, (48, 128), 0)
    l = lax.broadcasted_iota(jnp.int32, (48, 128), 1)
    slot = jnp.where(l >= 48, l - 48, l)
    xkey = (slot >= 16) & (l < 96)
    mkey = [(slot < 8) & (l < 96), (slot >= 8) & (slot < 16) & (l < 96)]
    xvalid = xkey & ((r < 16) | (r >= slot))
    valid = [xvalid | mkey[0], xvalid | mkey[1]]
    member = [xkey | mkey[0], xkey | mkey[1]]
    mem_h = [m_ & (l < 48) for m_ in member]
    mem_g = [m_ & (l >= 48) for m_ in member]
    lane_h = l < 48
    lane128 = lax.broadcasted_iota(jnp.int32, (80, 128), 1)
    lo = lane128 < 64
    fill = -1e9 / scale_a
    c_exp = scale_a * 1.4426950408889634

    def rows_c(a, c):
        return jnp.concatenate([a[0:16], a[16 + 32 * c:48 + 32 * c]], axis=0)

    def blk(a, c):
        a0, a1, a2 = a[:, 0:128], a[:, 128:256], a[:, 256:384]
        a1h = jnp.where(lo, a1, 0.0)
        a1g = jnp.where(lo, 0.0, a1)
        z = jnp.zeros((48, 128), F32)
        top = jnp.concatenate([rows_c(a0, c), rows_c(a1h, c), z], axis=1)
        mid = jnp.concatenate([z, rows_c(a1g, c), rows_c(a2, c)], axis=1)
        return jnp.concatenate([top, mid, jnp.zeros((32, PW), F32)], axis=0).astype(BF16)

    def rcp(x):
        r_ = pl.reciprocal(x, approx=True)
        return r_ * (2.0 - x * r_)

    def softmax_c(s, c):
        s = jnp.where(valid[c], s, fill)
        mh = jnp.max(jnp.where(mem_h[c], s, -jnp.inf), axis=-1, keepdims=True)
        mg = jnp.max(jnp.where(mem_g[c], s, -jnp.inf), axis=-1, keepdims=True)
        e = jnp.exp2((s - jnp.where(lane_h, mh, mg)) * c_exp)
        lh = jnp.sum(jnp.where(mem_h[c], e, 0.0), axis=-1, keepdims=True)
        lg = jnp.sum(jnp.where(mem_g[c], e, 0.0), axis=-1, keepdims=True)
        return (e * rcp(jnp.where(lane_h, lh, lg))).astype(BF16)

    def proj(h, w_ref, p):
        return _dot(h, w_ref[p * PW:(p + 1) * PW, :], NT)

    def qk(q, k):
        return [_dot(rows_c(q, c).astype(BF16), blk(k, c), NT) for c in range(2)]

    def pv(ss, v):
        os_ = [_dot(softmax_c(ss[c], c), blk(v, c)) for c in range(2)]
        return jnp.concatenate([os_[0][0:8], os_[1][8:16], os_[0][16:48], os_[1][16:48]], axis=0)

    def oproj(o, p):
        return _dot(o.astype(BF16), wo_ref[p * PW:(p + 1) * PW, :])

    def a_step(h, fill_work):
        acc = None
        k = proj(h, wk_ref, 0)
        o_prev = None
        for p in range(NP):
            q = proj(h, wq_ref, p)
            v = proj(h, wv_ref, p)
            ss = qk(q, k)
            if o_prev is not None:
                d = oproj(o_prev, p - 1)
                acc = d if acc is None else acc + d
            fill_work(p)
            if p + 1 < NP:
                k = proj(h, wk_ref, p + 1)
            o_prev = pv(ss, v)
        fill_work(NP)
        return acc + oproj(o_prev, NP - 1)

    rowi = lax.broadcasted_iota(jnp.int32, (SEG, 128), 0)

    def b_front():
        y = y_ref[...]
        return _dot(_ln(y).astype(BF16), bqkvp_ref[...])

    def b_attn(qkv, t):
        outs = []
        for lyr in range(2):
            seg = t - 1 - 2 * lyr
            q = qkv[32 * lyr:32 * lyr + 32, 0:D]
            kb_ref[lyr, 16:48, :] = qkv[32 * lyr:32 * lyr + 32, D:2 * D]
            vb_ref[lyr, 16:48, :] = qkv[32 * lyr:32 * lyr + 32, 2 * D:3 * D]
            logits = []
            for w in range(W):
                ks = kb_ref[lyr, 16 - DIL * w:48 - DIL * w, :]
                tt = q[:, 0:128] * ks[:, 0:128]
                for j in range(1, 5):
                    tt = tt + q[:, 128 * j:128 * j + 128] * ks[:, 128 * j:128 * j + 128]
                tt = tt + pltpu.roll(tt, 64, 1)
                tt = tt + pltpu.roll(tt, 32, 1)
                tt = tt * scale_b
                if w > 0:
                    tt = jnp.where(rowi + seg * SEG >= DIL * w, tt, -1e9)
                logits.append(tt)
            mx = functools.reduce(jnp.maximum, logits)
            es = [jnp.exp(t_ - mx) for t_ in logits]
            inv = rcp(functools.reduce(lambda a, b: a + b, es))
            o = None
            for w in range(W):
                a = es[w] * inv
                vs = vb_ref[lyr, 16 - DIL * w:48 - DIL * w, :]
                c = vs * jnp.concatenate([a] * 5, axis=1)
                o = c if o is None else o + c
            outs.append(o)
            kb_ref[lyr, 0:16, :] = kb_ref[lyr, 32:48, :]
            vb_ref[lyr, 0:16, :] = vb_ref[lyr, 32:48, :]
        return jnp.concatenate(outs, axis=0)

    def b_back(o):
        return y_ref[...] + _dot(o.astype(BF16), bwop_ref[...])

    def b_block(t):
        return b_back(b_attn(b_front(), t))

    def body(t, carry):
        h = h_ref[...]
        x2_res = x2_ref[...]
        st = {}

        def fill_work(p):
            if p == 0:
                st["qkv"] = b_front()
            elif p == 2:
                st["o"] = b_attn(st["qkv"], t)
            elif p == NP:
                st["z"] = b_back(st["o"])

        acc = a_step(h, fill_work)
        z = st["z"]
        x2_new = z[0:32]
        x2_ref[...] = x2_new
        h_ref[48:80, :] = _ln(x2_new).astype(BF16)
        to = jnp.maximum(t - 3, 0)
        out_ref[pl.ds(pl.multiple_of(to * SEG, SEG), SEG), :] = z[32:64].astype(out_ref.dtype)

        tn = jnp.minimum(t + 1, NSEG - 1)
        h_ref[16:48, :] = _ln(x_ref[pl.ds(pl.multiple_of(tn * SEG, SEG), SEG), :].astype(F32)).astype(BF16)

        m2 = jnp.where(t >= 2, acc[8:16], mem0)
        h_ref[0:16, :] = jnp.concatenate([acc[0:8], m2], axis=0).astype(BF16)
        tc = jnp.minimum(t, NSEG - 1)
        y_ref[0:32, :] = x_ref[pl.ds(pl.multiple_of(tc * SEG, SEG), SEG), :].astype(F32) + acc[16:48]
        y_ref[32:64, :] = x2_res + acc[48:80]
        return carry

    lax.fori_loop(0, NSEG + 2, body, 0)
    z = b_block(NSEG + 2)
    out_ref[pl.ds((NSEG - 1) * SEG, SEG), :] = z[32:64].astype(out_ref.dtype)


@functools.partial(jax.jit, static_argnames=("A_seg_len",))
def pallas_interleave_layers__memory_aug_recurrent_mem_tr__sliding_local_dilated__prompt_kernel(
    A_x: jax.Array,
    A_mem0: jax.Array,
    A_Wq: jax.Array,
    A_Wk: jax.Array,
    A_Wv: jax.Array,
    A_Wo: jax.Array,
    A_seg_len: int,
    B_x: jax.Array,
    B_wqkv: jax.Array,
    B_wo: jax.Array,
):
    del B_x
    B, S, D = A_x.shape
    _, H, DH = A_Wq.shape
    M = A_mem0.shape[1]
    SEG = int(A_seg_len)
    assert B == 1 and M == 8 and SEG == 32 and DH == 192 and D == 640

    x = A_x.reshape(S, D)
    mem0 = A_mem0.reshape(M, D)
    wq = A_Wq.transpose(1, 2, 0).reshape(H * DH, D)
    wk = A_Wk.transpose(1, 2, 0).reshape(H * DH, D)
    wv = A_Wv.transpose(1, 2, 0).reshape(H * DH, D)
    wo = A_Wo.reshape(H * DH, D)

    kern = functools.partial(_kernel, S=S, D=D, H=H, DH=DH, M=M, SEG=SEG, HB=32, W=8, DIL=2)
    out = pl.pallas_call(
        kern,
        out_shape=jax.ShapeDtypeStruct((S, D), A_x.dtype),
        scratch_shapes=[
            pltpu.VMEM((80, D), BF16),
            pltpu.VMEM((64, D), F32),
            pltpu.VMEM((SEG, D), F32),
            pltpu.VMEM((2, 48, D), F32),
            pltpu.VMEM((2, 48, D), F32),
            pltpu.VMEM((D, 3 * D), BF16),
            pltpu.VMEM((D, D), BF16),
        ],
        compiler_params=pltpu.CompilerParams(vmem_limit_bytes=110 * 1024 * 1024),
    )(x, mem0, wq, wk, wv, wo, B_wqkv, B_wo)
    return out.reshape(B, S, D)
```

```python
import functools


import jax
import jax.numpy as jnp
from jax import lax
import jax.experimental.pallas as pl
import jax.experimental.pallas.tpu as pltpu

F32 = jnp.float32
BF16 = jnp.bfloat16
U32 = jnp.uint32
NT = (((1,), (1,)), ((), ()))
NN = (((1,), (0,)), ((), ()))
LOG2E = 1.4426950408889634

CFG = dict(wo0=7, bf=0, lnx=3, unroll=1, ob16=0, win=4)
for kv in "".split(","):
    if kv:
        k_, v_ = kv.split("=")
        CFG[k_] = int(v_)


def _ln(x):
    m = jnp.mean(x, axis=-1, keepdims=True)
    xc = x - m
    v = jnp.mean(xc * xc, axis=-1, keepdims=True)
    return xc * lax.rsqrt(v + 1e-5)


def _dot(a, b, dims=NN):
    return lax.dot_general(a, b, dims, preferred_element_type=F32)


def _rcp(x):
    r_ = pl.reciprocal(x, approx=True)
    return r_ * (2.0 - x * r_)


def _kernel(x_hbm, mem0_ref, wq_hbm, wk_hbm, wv_hbm, wo_hbm, bqkv_hbm, bwo_hbm,
            out_hbm,
            x_ref, out_ref, lq_ref, lk_ref, lv_ref, lo_ref, wq_ref, wk_ref, wv_ref, wo_ref,
            lbqkv_ref, lbwo_ref, bqf_ref, bof_ref, bqkvp_ref, bwop_ref,
            h_ref, y_ref, x2_ref, kb_ref, vb_ref, sem,
            *, S, D, H, DH, M, SEG, HB, W, DIL):
    NSEG = S // SEG
    NP = H // 2
    PW = 2 * DH
    scale_a = DH ** -0.5
    DHB = D // HB
    scale_b = DHB ** -0.5
    NTB = D // 128
    XH = 4 * SEG
    WIN = CFG["win"]

    def w_copy(m, p):
        src, dst = ((wk_hbm, lk_ref), (wq_hbm, lq_ref), (wv_hbm, lv_ref), (wo_hbm, lo_ref))[m]
        rows = pl.ds(pl.multiple_of(p * PW, PW), PW)
        return pltpu.make_async_copy(src.at[rows, :], dst.at[rows, :], sem.at[4 * p + m])

    c_x = pltpu.make_async_copy(x_hbm, x_ref, sem.at[4 * NP])
    c_bq = pltpu.make_async_copy(bqkv_hbm, lbqkv_ref, sem.at[4 * NP + 1])
    c_bo = pltpu.make_async_copy(bwo_hbm, lbwo_ref, sem.at[4 * NP + 2])
    S1 = (NSEG - 3) * SEG
    c_o1 = pltpu.make_async_copy(out_ref.at[pl.ds(0, S1), :], out_hbm.at[pl.ds(0, S1), :], sem.at[4 * NP + 3])
    c_o2 = pltpu.make_async_copy(out_ref.at[pl.ds(S1, S - S1), :], out_hbm.at[pl.ds(S1, S - S1), :], sem.at[4 * NP + 4])

    def issue(p):
        for m in range(4):
            w_copy(m, p).start()

    c_bq.start()
    c_bo.start()
    for p in range(WIN):
        issue(p)

    mem0 = mem0_ref[...].astype(F32)
    h_ref[0:16, :] = jnp.concatenate([mem0, mem0], axis=0).astype(BF16)
    h_ref[48:80, :] = jnp.zeros((SEG, D), BF16)
    y_ref[...] = jnp.zeros(y_ref.shape, F32)
    x2_ref[...] = jnp.zeros(x2_ref.shape, F32)
    kb_ref[...] = jnp.zeros(kb_ref.shape, F32)
    vb_ref[...] = jnp.zeros(vb_ref.shape, F32)
    c_bq.wait()
    c_bo.wait()

    RB = D // NP

    def conv_body(p, carry):
        for m in range(4):
            w_copy(m, p).wait()

        @pl.when(p + WIN < NP)
        def _():
            issue(p + WIN)

        @pl.when(p + WIN == NP)
        def _():
            c_x.start()

        rows = pl.ds(pl.multiple_of(p * PW, PW), PW)
        wk_ref[p] = pltpu.bitcast(lk_ref[rows, :].T, U32)
        wq_ref[p] = pltpu.bitcast(lq_ref[rows, :].T, U32)
        wv_ref[p] = pltpu.bitcast(lv_ref[rows, :].T, U32)
        wo_ref[p] = pltpu.bitcast(lo_ref[rows, :], U32)
        ri = lax.broadcasted_iota(jnp.int32, (D, D), 0)
        ci = lax.broadcasted_iota(jnp.int32, (D, D), 1)
        pm = (ri == (ci % HB) * DHB + ci // HB).astype(BF16)
        brow = pl.ds(pl.multiple_of(p * RB, 8), RB)
        r4 = lax.broadcasted_iota(jnp.int32, (RB, D), 0) + p * RB
        c4 = lax.broadcasted_iota(jnp.int32, (RB, D), 1)
        pmt = (c4 == (r4 % HB) * DHB + r4 // HB).astype(F32)
        for j in range(3):
            bqf_ref[brow, j * D:(j + 1) * D] = _dot(lbqkv_ref[brow, j * D:(j + 1) * D].astype(F32), pm)
        bof_ref[brow, :] = _dot(pmt, lbwo_ref[...])
        return carry

    lax.fori_loop(0, NP, conv_body, 0)
    bqkvp_ref[...] = pltpu.bitcast(bqf_ref[...].astype(BF16), U32)
    bwop_ref[...] = pltpu.bitcast(bof_ref[...].astype(BF16), U32)
    c_x.wait()
    h_ref[16:48, :] = _ln(x_ref[0:SEG, :].astype(F32)).astype(BF16)

    L = M + SEG
    r = lax.broadcasted_iota(jnp.int32, (L, 128), 0)
    l = lax.broadcasted_iota(jnp.int32, (L, 128), 1)
    slot = jnp.where(l >= L, l - L, l)
    valid = (l < 2 * L) & ((r < M) | (r >= slot))
    in_h = l < L
    in_g = (l >= L) & (l < 2 * L)
    lo = l < 64
    fill = -1e9 / scale_a
    c_exp = scale_a * LOG2E

    def rows_c(a, c):
        if a.shape[0] == L:
            return a
        return jnp.concatenate([a[M * c:M * c + M], a[16 + SEG * c:16 + SEG * c + SEG]], axis=0)

    def blk(a, c, pad):
        a = rows_c(a, c)
        a0, a1, a2 = a[:, 0:128], a[:, 128:256], a[:, 256:384]
        z = jnp.zeros((L, 128), F32)
        top = jnp.concatenate([a0, jnp.where(lo, a1, 0.0), z], axis=1)
        bot = jnp.concatenate([z, jnp.where(lo, 0.0, a1), a2], axis=1)
        parts = [top, bot] + ([jnp.zeros((128 - 2 * L, PW), F32)] if pad else [])
        return jnp.concatenate(parts, axis=0).astype(BF16)

    def proj(h, w_ref, p):
        return _dot(h, pltpu.bitcast(w_ref[p], BF16))

    def qk(q, k, chains):
        return [_dot(rows_c(q, c), blk(k, c, False), NT) for c in chains]

    def attn_c(s, v, c):
        s = jnp.concatenate([s, jnp.full((L, 128 - 2 * L), fill, F32)], axis=1)
        s = jnp.where(valid, s, fill)
        mh = jnp.max(jnp.where(in_h, s, -jnp.inf), axis=-1, keepdims=True)
        mg = jnp.max(jnp.where(in_g, s, -jnp.inf), axis=-1, keepdims=True)
        e = jnp.exp2((s - jnp.where(in_h, mh, mg)) * c_exp)
        e = jnp.where(l < 2 * L, e, 0.0)
        ih = _rcp(jnp.sum(jnp.where(in_h, e, 0.0), axis=-1, keepdims=True))
        ig = _rcp(jnp.sum(jnp.where(in_g, e, 0.0), axis=-1, keepdims=True))
        o = _dot(e, blk(v, c, True))
        return jnp.concatenate([o[:, 0:128] * ih, o[:, 128:256] * jnp.where(lo, ih, ig), o[:, 256:384] * ig], axis=1)

    def pv(ss, v, chains):
        os_ = [attn_c(s, v, c) for s, c in zip(ss, chains)]
        if len(chains) == 2:
            o = jnp.concatenate([os_[0][0:M], os_[1][0:M], os_[0][M:L], os_[1][M:L]], axis=0)
            return o.astype(BF16) if CFG["ob16"] else o
        return os_[0]

    def oproj(o, p):
        return _dot(o, pltpu.bitcast(wo_ref[p], BF16))

    rowi = lax.broadcasted_iota(jnp.int32, (16, 128), 0)
    fill_b = -1e9 / scale_b
    c_expb = scale_b * LOG2E

    def b_front():
        qkv = _dot(_ln(y_ref[...]).astype(BF16), pltpu.bitcast(bqkvp_ref[...], BF16))
        for lyr in range(2):
            for j in range(NTB):
                kb_ref[lyr, j, 16:48, :] = qkv[32 * lyr:32 * lyr + 32, D + 128 * j:D + 128 * j + 128]
                vb_ref[lyr, j, 16:48, :] = qkv[32 * lyr:32 * lyr + 32, 2 * D + 128 * j:2 * D + 128 * j + 128]
        return qkv[:, 0:D]

    def b_attn(q, t, lyr):
        seg = t - 1 - 2 * lyr
        q = q[32 * lyr:32 * lyr + 32]
        logits = []
        for w in range(W):
            tt = None
            for j in range(NTB):
                pr = q[:, 128 * j:128 * j + 128] * kb_ref[lyr, j, 16 - DIL * w:48 - DIL * w, :]
                tt = pr if tt is None else tt + pr
            tt = tt + pltpu.roll(tt, 64, 1)
            tt = tt + pltpu.roll(tt, 32, 1)
            if w > 0:
                top = jnp.where(rowi >= DIL * w - seg * SEG, tt[0:16], fill_b)
                tt = jnp.concatenate([top, tt[16:32]], axis=0)
            logits.append(tt)
        mx = functools.reduce(jnp.maximum, logits)
        es = [jnp.exp2((t_ - mx) * c_expb) for t_ in logits]
        inv = _rcp(functools.reduce(lambda a, b: a + b, es))
        outs = []
        for j in range(NTB):
            o = None
            for w in range(W):
                c = es[w] * vb_ref[lyr, j, 16 - DIL * w:48 - DIL * w, :]
                o = c if o is None else o + c
            outs.append(o * inv)
        for j in range(NTB):
            kb_ref[lyr, j, 0:16, :] = kb_ref[lyr, j, 32:48, :]
            vb_ref[lyr, j, 0:16, :] = vb_ref[lyr, j, 32:48, :]
        return jnp.concatenate(outs, axis=1)

    def b_back(o, lyr):
        return y_ref[32 * lyr:32 * lyr + 32, :] + _dot(o, pltpu.bitcast(bwop_ref[...], BF16))

    def seg_rows(s):
        if isinstance(s, int):
            return pl.ds(s * SEG, SEG)
        return pl.ds(pl.multiple_of(s * SEG, SEG), SEG)

    def step(t, chains=(0, 1)):
        dual = len(chains) == 2
        if dual:
            h = h_ref[...]
        else:
            h = rows_c(h_ref[...].astype(F32), chains[0])
        x2_res = x2_ref[...] if 1 in chains else None
        st = {}

        def b0():
            z = b_back(b_attn(st["q"], t, 0), 0)
            x2_ref[...] = z
            h_ref[48:80, :] = _ln(z).astype(BF16)

        def b1():
            z = b_back(b_attn(st["q"], t, 1), 1)
            out_ref[seg_rows(jnp.maximum(t - 3, 0)), :] = z.astype(out_ref.dtype)

        def prj(m, p):
            return proj(h, (wk_ref, wq_ref, wv_ref)[m], p)

        opj = oproj

        k = prj(0, 0)
        q = prj(1, 0)
        v = prj(2, 0)
        acc = None
        o_prev = None
        for p in range(NP):
            ss = qk(q, k, chains)
            if p == CFG["bf"]:
                st["q"] = b_front()
            if p == CFG["lnx"] and 0 in chains:
                tn = jnp.minimum(t + 1, NSEG - 1)
                h_ref[16:48, :] = _ln(x_ref[seg_rows(tn), :].astype(F32)).astype(BF16)
            if p + 1 < NP:
                q = prj(1, p + 1)
                k = prj(0, p + 1)
            else:
                acc = acc + opj(o_prev, p - 1)
            o = pv(ss, v, chains)
            if p + 1 < NP:
                v = prj(2, p + 1)
            elif 1 in chains:
                b1()
            if p != NP - 2:
                d = opj(o, p)
                acc = d if acc is None else acc + d
            o_prev = o
            if p == CFG["wo0"]:
                b0()

        if dual:
            h_ref[0:16, :] = acc[0:16].astype(BF16)
            y_ref[0:32, :] = x_ref[seg_rows(t), :].astype(F32) + acc[16:48]
            y_ref[32:64, :] = x2_res + acc[48:80]
        elif chains[0] == 0:
            h_ref[0:M, :] = acc[0:M].astype(BF16)
            y_ref[0:32, :] = x_ref[seg_rows(t), :].astype(F32) + acc[M:L]
        else:
            h_ref[M:2 * M, :] = acc[0:M].astype(BF16)
            y_ref[32:64, :] = x2_res + acc[M:L]

    def run(lo_, hi_, chains, unroll=1):
        def body(i, carry):
            for u in range(unroll):
                step(lo_ + i * unroll + u, chains)
            return carry
        lax.fori_loop(0, (hi_ - lo_) // unroll, body, 0)

    run(0, 2, (0,))
    run(2, 2 + CFG.get("nit", NSEG - 2), (0, 1), CFG["unroll"])
    c_o1.start()
    run(NSEG, NSEG + 2, (1,))
    z = b_back(b_attn(b_front(), NSEG + 2, 1), 1)
    out_ref[seg_rows(NSEG - 1), :] = z.astype(out_ref.dtype)
    c_o2.start()
    c_o1.wait()
    c_o2.wait()


@functools.partial(jax.jit, static_argnames=("A_seg_len",))
def pallas_interleave_layers__memory_aug_recurrent_mem_tr__sliding_local_dilated__prompt_kernel(
    A_x, A_mem0, A_Wq, A_Wk, A_Wv, A_Wo, A_seg_len, B_x, B_wqkv, B_wo,
):
    del B_x
    B, S, D = A_x.shape
    _, H, DH = A_Wq.shape
    M = A_mem0.shape[1]
    SEG = int(A_seg_len)
    assert B == 1 and M == 8 and SEG == 32 and DH == 192 and D == 640
    NP, PW = H // 2, 2 * DH

    x = A_x.reshape(S, D)
    mem0 = A_mem0.reshape(M, D)
    wq = A_Wq.transpose(1, 2, 0).reshape(H * DH, D)
    wk = A_Wk.transpose(1, 2, 0).reshape(H * DH, D)
    wv = A_Wv.transpose(1, 2, 0).reshape(H * DH, D)
    wo = A_Wo.reshape(H * DH, D)

    kern = functools.partial(_kernel, S=S, D=D, H=H, DH=DH, M=M, SEG=SEG, HB=32, W=8, DIL=2)
    hbm = pl.BlockSpec(memory_space=pl.ANY)
    out = pl.pallas_call(
        kern,
        out_shape=jax.ShapeDtypeStruct((S, D), A_x.dtype),
        in_specs=[hbm, pl.BlockSpec(memory_space=pltpu.VMEM), hbm, hbm, hbm, hbm, hbm, hbm],
        out_specs=hbm,
        scratch_shapes=[
            pltpu.VMEM((S, D), BF16),
            pltpu.VMEM((S, D), A_x.dtype),
            pltpu.VMEM((H * DH, D), BF16),
            pltpu.VMEM((H * DH, D), BF16),
            pltpu.VMEM((H * DH, D), BF16),
            pltpu.VMEM((H * DH, D), BF16),
            pltpu.VMEM((NP, D // 2, PW), U32),
            pltpu.VMEM((NP, D // 2, PW), U32),
            pltpu.VMEM((NP, D // 2, PW), U32),
            pltpu.VMEM((NP, PW // 2, D), U32),
            pltpu.VMEM((D, 3 * D), BF16),
            pltpu.VMEM((D, D), BF16),
            pltpu.VMEM((D, 3 * D), F32),
            pltpu.VMEM((D, D), F32),
            pltpu.VMEM((D // 2, 3 * D), U32),
            pltpu.VMEM((D // 2, D), U32),
            pltpu.VMEM((80, D), BF16),
            pltpu.VMEM((64, D), F32),
            pltpu.VMEM((SEG, D), F32),
            pltpu.VMEM((2, D // 128, 48, 128), F32),
            pltpu.VMEM((2, D // 128, 48, 128), F32),
            pltpu.SemaphoreType.DMA((4 * NP + 5,)),
        ],
        compiler_params=pltpu.CompilerParams(vmem_limit_bytes=110 * 1024 * 1024),
    )(x, mem0, wq, wk, wv, wo, B_wqkv, B_wo)
    return out.reshape(B, S, D)
```

```python
import functools

import jax
import jax.numpy as jnp
from jax import lax
import jax.experimental.pallas as pl
import jax.experimental.pallas.tpu as pltpu

F32 = jnp.float32
BF16 = jnp.bfloat16
U32 = jnp.uint32
NT = (((1,), (1,)), ((), ()))
NN = (((1,), (0,)), ((), ()))
LOG2E = 1.4426950408889634

CFG = dict(wo0=7, bf=0, lnx=9, win=4, nit=62, vsplit=1)


def _ln(x):
    m = jnp.mean(x, axis=-1, keepdims=True)
    xc = x - m
    v = jnp.mean(xc * xc, axis=-1, keepdims=True)
    return xc * lax.rsqrt(v + 1e-5)


def _dot(a, b, dims=NN):
    return lax.dot_general(a, b, dims, preferred_element_type=F32)


def _rcp(x):
    r_ = pl.reciprocal(x, approx=True)
    return r_ * (2.0 - x * r_)


def _pack(x):
    return pltpu.bitcast(x, U32)


def _unpack(x):
    return pltpu.bitcast(x, BF16)


def _kernel(x_hbm, mem0_ref, wq_hbm, wk_hbm, wv_hbm, wo_hbm, bqkv_hbm, bwo_hbm,
            out_hbm,
            x_ref, out_ref, lq_ref, lk_ref, lv_ref, lo_ref, wq_ref, wk_ref, wv_ref, wo_ref,
            lbqkv_ref, lbwo_ref, bqf_ref, bof_ref, bqkvp_ref, bwop_ref,
            h_ref, y_ref, x2_ref, kb_ref, vb_ref, h0_ref, acc0_ref, sem,
            *, S, D, H, DH, M, SEG, HB, W, DIL):
    NSEG = S // SEG
    NP = H // 2
    PW = 2 * DH
    L = M + SEG
    scale_a = DH ** -0.5
    DHB = D // HB
    scale_b = DHB ** -0.5
    NTB = D // 128
    XH = 4 * SEG
    WIN = CFG["win"]

    def w_copy(m, p):
        src, dst = ((wk_hbm, lk_ref), (wq_hbm, lq_ref), (wv_hbm, lv_ref), (wo_hbm, lo_ref))[m]
        rows = pl.ds(pl.multiple_of(p * PW, PW), PW)
        return pltpu.make_async_copy(src.at[rows, :], dst.at[rows, :], sem.at[4 * p + m])

    c_xh = pltpu.make_async_copy(x_hbm.at[pl.ds(0, XH), :], x_ref.at[pl.ds(0, XH), :], sem.at[4 * NP])
    c_xr = pltpu.make_async_copy(x_hbm.at[pl.ds(XH, S - XH), :], x_ref.at[pl.ds(XH, S - XH), :], sem.at[4 * NP + 1])
    c_bq = pltpu.make_async_copy(bqkv_hbm, lbqkv_ref, sem.at[4 * NP + 2])
    c_bo = pltpu.make_async_copy(bwo_hbm, lbwo_ref, sem.at[4 * NP + 3])
    S1 = (NSEG - 3) * SEG
    c_o1 = pltpu.make_async_copy(out_ref.at[pl.ds(0, S1), :], out_hbm.at[pl.ds(0, S1), :], sem.at[4 * NP + 4])
    c_o2 = pltpu.make_async_copy(out_ref.at[pl.ds(S1, S - S1), :], out_hbm.at[pl.ds(S1, S - S1), :], sem.at[4 * NP + 5])

    def issue(p):
        for m in range(4):
            w_copy(m, p).start()

    c_xh.start()
    c_bq.start()
    c_bo.start()
    for p in range(WIN):
        issue(p)

    r = lax.broadcasted_iota(jnp.int32, (L, 128), 0)
    l = lax.broadcasted_iota(jnp.int32, (L, 128), 1)
    slot = jnp.where(l >= L, l - L, l)
    valid = (l < 2 * L) & ((r < M) | (r >= slot))
    in_h = l < L
    in_g = (l >= L) & (l < 2 * L)
    lo = l < 64
    fill = -1e9 / scale_a
    c_exp = scale_a * LOG2E

    def rows_c(a, c):
        if a.shape[0] == L:
            return a
        return jnp.concatenate([a[M * c:M * c + M], a[2 * M + SEG * c:2 * M + SEG * c + SEG]], axis=0)

    def blk(a, c, pad):
        a = rows_c(a, c)
        a0, a1, a2 = a[:, 0:128], a[:, 128:256], a[:, 256:384]
        z = jnp.zeros((L, 128), F32)
        top = jnp.concatenate([a0, jnp.where(lo, a1, 0.0), z], axis=1)
        bot = jnp.concatenate([z, jnp.where(lo, 0.0, a1), a2], axis=1)
        parts = [top, bot] + ([jnp.zeros((128 - 2 * L, PW), F32)] if pad else [])
        return jnp.concatenate(parts, axis=0).astype(BF16)

    def qk(q, k, chains):
        return [_dot(rows_c(q, c), blk(k, c, False), NT) for c in chains]

    def attn_c(s, v, c):
        s = jnp.concatenate([s, jnp.full((L, 128 - 2 * L), fill, F32)], axis=1)
        s = jnp.where(valid, s, fill)
        mh = jnp.max(jnp.where(in_h, s, -jnp.inf), axis=-1, keepdims=True)
        mg = jnp.max(jnp.where(in_g, s, -jnp.inf), axis=-1, keepdims=True)
        e = jnp.exp2((s - jnp.where(in_h, mh, mg)) * c_exp)
        e = jnp.where(l < 2 * L, e, 0.0)
        ih = _rcp(jnp.sum(jnp.where(in_h, e, 0.0), axis=-1, keepdims=True))
        ig = _rcp(jnp.sum(jnp.where(in_g, e, 0.0), axis=-1, keepdims=True))
        o = _dot(e, blk(v, c, True))
        return jnp.concatenate([o[:, 0:128] * ih, o[:, 128:256] * jnp.where(lo, ih, ig), o[:, 256:384] * ig], axis=1)

    def pv(ss, v, chains):
        os_ = [attn_c(s, v, c) for s, c in zip(ss, chains)]
        if len(chains) == 2:
            return jnp.concatenate([os_[0][0:M], os_[1][0:M], os_[0][M:L], os_[1][M:L]], axis=0)
        return os_[0]

    def seg_rows(s):
        if isinstance(s, int):
            return pl.ds(s * SEG, SEG)
        return pl.ds(pl.multiple_of(s * SEG, SEG), SEG)

    mem0 = mem0_ref[...]
    y_ref[...] = jnp.zeros(y_ref.shape, F32)
    x2_ref[...] = jnp.zeros(x2_ref.shape, F32)
    kb_ref[...] = jnp.zeros(kb_ref.shape, F32)
    vb_ref[...] = jnp.zeros(vb_ref.shape, F32)
    acc0_ref[...] = jnp.zeros(acc0_ref.shape, F32)
    c_xh.wait()
    h0_ref[0:M, :] = mem0.astype(F32)
    h0_ref[M:L, :] = _ln(x_ref[0:SEG, :].astype(F32)).astype(BF16).astype(F32)

    RB = D // NP

    def conv_body(p, carry):
        for m in range(4):
            w_copy(m, p).wait()

        @pl.when(p + WIN < NP)
        def _():
            issue(p + WIN)

        @pl.when(p + WIN == NP)
        def _():
            c_xr.start()

        rows = pl.ds(pl.multiple_of(p * PW, PW), PW)
        h = h0_ref[...]
        wk = lk_ref[rows, :].T
        wq = lq_ref[rows, :].T
        wv = lv_ref[rows, :].T
        wo = lo_ref[rows, :]
        wk_ref[p] = _pack(wk)
        wq_ref[p] = _pack(wq)
        wv_ref[p] = _pack(wv)
        wo_ref[p] = _pack(wo)
        k = _dot(h, wk)
        q = _dot(h, wq)
        v = _dot(h, wv)
        ss = qk(q, k, (0,))
        ri = lax.broadcasted_iota(jnp.int32, (D, D), 0)
        ci = lax.broadcasted_iota(jnp.int32, (D, D), 1)
        pm = (ri == (ci % HB) * DHB + ci // HB).astype(BF16)
        brow = pl.ds(pl.multiple_of(p * RB, 8), RB)
        r4 = lax.broadcasted_iota(jnp.int32, (RB, D), 0) + p * RB
        c4 = lax.broadcasted_iota(jnp.int32, (RB, D), 1)
        pmt = (c4 == (r4 % HB) * DHB + r4 // HB).astype(F32)
        for j in range(2):
            bqf_ref[brow, j * D:(j + 1) * D] = _dot(lbqkv_ref[brow, j * D:(j + 1) * D].astype(F32), pm)
        o = pv(ss, v, (0,))
        bqf_ref[brow, 2 * D:3 * D] = _dot(lbqkv_ref[brow, 2 * D:3 * D].astype(F32), pm)
        acc0_ref[...] += _dot(o, wo)
        bof_ref[brow, :] = _dot(pmt, lbwo_ref[...])
        return carry

    c_bq.wait()
    c_bo.wait()
    lax.fori_loop(0, NP, conv_body, 0)
    bqkvp_ref[...] = _pack(bqf_ref[...].astype(BF16))
    bwop_ref[...] = _pack(bof_ref[...].astype(BF16))
    acc0 = acc0_ref[...]
    h_ref[0:2 * M, :] = jnp.concatenate([acc0[0:M], mem0.astype(F32)], axis=0).astype(BF16)
    h_ref[2 * M:2 * M + SEG, :] = _ln(x_ref[seg_rows(1), :].astype(F32)).astype(BF16)
    h_ref[2 * M + SEG:2 * L, :] = jnp.zeros((SEG, D), BF16)
    y_ref[0:SEG, :] = x_ref[seg_rows(0), :].astype(F32) + acc0[M:L]

    rowi = lax.broadcasted_iota(jnp.int32, (16, 128), 0)
    fill_b = -1e9 / scale_b
    c_expb = scale_b * LOG2E

    def b_front():
        qkv = _dot(_ln(y_ref[...]).astype(BF16), _unpack(bqkvp_ref[...]))
        for lyr in range(2):
            for j in range(NTB):
                kb_ref[lyr, j, 16:48, :] = qkv[32 * lyr:32 * lyr + 32, D + 128 * j:D + 128 * j + 128]
                vb_ref[lyr, j, 16:48, :] = qkv[32 * lyr:32 * lyr + 32, 2 * D + 128 * j:2 * D + 128 * j + 128]
        return qkv[:, 0:D]

    def b_attn(q, t, lyr):
        seg = t - 1 - 2 * lyr
        q = q[32 * lyr:32 * lyr + 32]
        logits = []
        for w in range(W):
            tt = None
            for j in range(NTB):
                pr = q[:, 128 * j:128 * j + 128] * kb_ref[lyr, j, 16 - DIL * w:48 - DIL * w, :]
                tt = pr if tt is None else tt + pr
            tt = tt + pltpu.roll(tt, 64, 1)
            tt = tt + pltpu.roll(tt, 32, 1)
            if w > 0:
                top = jnp.where(rowi >= DIL * w - seg * SEG, tt[0:16], fill_b)
                tt = jnp.concatenate([top, tt[16:32]], axis=0)
            logits.append(tt)
        mx = functools.reduce(jnp.maximum, logits)
        es = [jnp.exp2((t_ - mx) * c_expb) for t_ in logits]
        inv = _rcp(functools.reduce(lambda a, b: a + b, es))
        outs = []
        for j in range(NTB):
            o = None
            for w in range(W):
                c = es[w] * vb_ref[lyr, j, 16 - DIL * w:48 - DIL * w, :]
                o = c if o is None else o + c
            outs.append(o * inv)
        for j in range(NTB):
            kb_ref[lyr, j, 0:16, :] = kb_ref[lyr, j, 32:48, :]
            vb_ref[lyr, j, 0:16, :] = vb_ref[lyr, j, 32:48, :]
        return jnp.concatenate(outs, axis=1)

    def b_back(o, lyr):
        return y_ref[32 * lyr:32 * lyr + 32, :] + _dot(o, _unpack(bwop_ref[...]))

    def step(t, chains):
        dual = len(chains) == 2
        if dual:
            h = h_ref[...]
        else:
            h = rows_c(h_ref[...].astype(F32), chains[0])
        x2_res = x2_ref[...] if 1 in chains else None
        st = {}

        def b0():
            z = b_back(b_attn(st["q"], t, 0), 0)
            x2_ref[...] = z
            h_ref[2 * M + SEG:2 * L, :] = _ln(z).astype(BF16)

        def b1():
            z = b_back(b_attn(st["q"], t, 1), 1)
            out_ref[seg_rows(jnp.maximum(t - 3, 0)), :] = z.astype(out_ref.dtype)

        def prj(w_ref, p, cols=slice(None)):
            return _dot(h, _unpack(w_ref[p, :, cols]))

        def opj(o, p):
            return _dot(o, _unpack(wo_ref[p]))

        k = prj(wk_ref, 0)
        q = prj(wq_ref, 0)
        v = prj(wv_ref, 0)
        acc = None
        for p in range(NP):
            ss = qk(q, k, chains)
            if p == CFG["bf"]:
                st["q"] = b_front()
            if p == CFG["lnx"] and 0 in chains:
                tn = jnp.minimum(t + 1, NSEG - 1)
                h_ref[2 * M:2 * M + SEG, :] = _ln(x_ref[seg_rows(tn), :].astype(F32)).astype(BF16)
            if p + 1 < NP:
                q = prj(wq_ref, p + 1)
                k = prj(wk_ref, p + 1)
            else:
                if CFG["vsplit"]:
                    v = jnp.concatenate([v, prj(wv_ref, p, slice(256, 384))], axis=1)
                acc = acc + opj(o, p - 1)
            o = pv(ss, v, chains)
            if p + 2 < NP:
                v = prj(wv_ref, p + 1)
            elif p + 2 == NP:
                v = prj(wv_ref, p + 1, slice(0, 256)) if CFG["vsplit"] else prj(wv_ref, p + 1)
            elif 1 in chains:
                b1()
            if p != NP - 2:
                d = opj(o, p)
                acc = d if acc is None else acc + d
            if p == CFG["wo0"]:
                b0()

        if dual:
            h_ref[0:2 * M, :] = acc[0:2 * M].astype(BF16)
            y_ref[0:SEG, :] = x_ref[seg_rows(t), :].astype(F32) + acc[2 * M:2 * M + SEG]
            y_ref[SEG:2 * SEG, :] = x2_res + acc[2 * M + SEG:2 * L]
        elif chains[0] == 0:
            h_ref[0:M, :] = acc[0:M].astype(BF16)
            y_ref[0:SEG, :] = x_ref[seg_rows(t), :].astype(F32) + acc[M:L]
        else:
            h_ref[M:2 * M, :] = acc[0:M].astype(BF16)
            y_ref[SEG:2 * SEG, :] = x2_res + acc[M:L]

    def run(lo_, hi_, chains):
        def body(t, carry):
            step(t, chains)
            return carry
        lax.fori_loop(lo_, hi_, body, 0)

    run(1, 2, (0,))
    c_xr.wait()
    run(2, 2 + CFG["nit"], (0, 1))
    c_o1.start()
    run(NSEG, NSEG + 2, (1,))
    z = b_back(b_attn(b_front(), NSEG + 2, 1), 1)
    out_ref[seg_rows(NSEG - 1), :] = z.astype(out_ref.dtype)
    c_o2.start()
    c_o1.wait()
    c_o2.wait()


@functools.partial(jax.jit, static_argnames=("A_seg_len",))
def pallas_interleave_layers__memory_aug_recurrent_mem_tr__sliding_local_dilated__prompt_kernel(
    A_x, A_mem0, A_Wq, A_Wk, A_Wv, A_Wo, A_seg_len, B_x, B_wqkv, B_wo,
):
    del B_x
    B, S, D = A_x.shape
    _, H, DH = A_Wq.shape
    M = A_mem0.shape[1]
    SEG = int(A_seg_len)
    assert B == 1 and M == 8 and SEG == 32 and DH == 192 and D == 640
    NP, PW = H // 2, 2 * DH

    x = A_x.reshape(S, D)
    mem0 = A_mem0.reshape(M, D)
    wq = A_Wq.transpose(1, 2, 0).reshape(H * DH, D)
    wk = A_Wk.transpose(1, 2, 0).reshape(H * DH, D)
    wv = A_Wv.transpose(1, 2, 0).reshape(H * DH, D)
    wo = A_Wo.reshape(H * DH, D)

    kern = functools.partial(_kernel, S=S, D=D, H=H, DH=DH, M=M, SEG=SEG, HB=32, W=8, DIL=2)
    hbm = pl.BlockSpec(memory_space=pl.ANY)
    out = pl.pallas_call(
        kern,
        out_shape=jax.ShapeDtypeStruct((S, D), A_x.dtype),
        in_specs=[hbm, pl.BlockSpec(memory_space=pltpu.VMEM), hbm, hbm, hbm, hbm, hbm, hbm],
        out_specs=hbm,
        scratch_shapes=[
            pltpu.VMEM((S, D), BF16),
            pltpu.VMEM((S, D), A_x.dtype),
            pltpu.VMEM((H * DH, D), BF16),
            pltpu.VMEM((H * DH, D), BF16),
            pltpu.VMEM((H * DH, D), BF16),
            pltpu.VMEM((H * DH, D), BF16),
            pltpu.VMEM((NP, D // 2, PW), U32),
            pltpu.VMEM((NP, D // 2, PW), U32),
            pltpu.VMEM((NP, D // 2, PW), U32),
            pltpu.VMEM((NP, PW // 2, D), U32),
            pltpu.VMEM((D, 3 * D), BF16),
            pltpu.VMEM((D, D), BF16),
            pltpu.VMEM((D, 3 * D), F32),
            pltpu.VMEM((D, D), F32),
            pltpu.VMEM((D // 2, 3 * D), U32),
            pltpu.VMEM((D // 2, D), U32),
            pltpu.VMEM((2 * (M + SEG), D), BF16),
            pltpu.VMEM((2 * SEG, D), F32),
            pltpu.VMEM((SEG, D), F32),
            pltpu.VMEM((2, D // 128, 48, 128), F32),
            pltpu.VMEM((2, D // 128, 48, 128), F32),
            pltpu.VMEM((M + SEG, D), F32),
            pltpu.VMEM((M + SEG, D), F32),
            pltpu.SemaphoreType.DMA((4 * NP + 6,)),
        ],
        compiler_params=pltpu.CompilerParams(vmem_limit_bytes=110 * 1024 * 1024),
    )(x, mem0, wq, wk, wv, wo, B_wqkv, B_wo)
    return out.reshape(B, S, D)
```

```python
import functools

import jax
import jax.numpy as jnp
from jax import lax
import jax.experimental.pallas as pl
import jax.experimental.pallas.tpu as pltpu

F32 = jnp.float32
BF16 = jnp.bfloat16
U32 = jnp.uint32
NT = (((1,), (1,)), ((), ()))
NN = (((1,), (0,)), ((), ()))
LOG2E = 1.4426950408889634

CFG = dict(wo0=7, bf=0, lnx=9, win=4, nit=62, vsplit=1, npre=8, pb=3)


def _ln(x):
    m = jnp.mean(x, axis=-1, keepdims=True)
    xc = x - m
    v = jnp.mean(xc * xc, axis=-1, keepdims=True)
    return xc * lax.rsqrt(v + 1e-5)


def _dot(a, b, dims=NN):
    return lax.dot_general(a, b, dims, preferred_element_type=F32)


def _rcp(x):
    r_ = pl.reciprocal(x, approx=True)
    return r_ * (2.0 - x * r_)


def _pack(x):
    return pltpu.bitcast(x, U32)


def _unpack(x):
    return pltpu.bitcast(x, BF16)


def _kernel(x_hbm, mem0_ref, wq_hbm, wk_hbm, wv_hbm, wo_hbm, bqkv_hbm, bwo_hbm,
            out_hbm,
            x_ref, out_ref, lq_ref, lk_ref, lv_ref, lo_ref, wq_ref, wk_ref, wv_ref, wo_ref,
            lbqkv_ref, lbwo_ref, tf_ref, bqkvp_ref, bwop_ref,
            h_ref, y_ref, x2_ref, kb_ref, vb_ref, h0_ref, acc0_ref, qp_ref, kp_ref, vp_ref, sem,
            *, S, D, H, DH, M, SEG, HB, W, DIL):
    NSEG = S // SEG
    NP = H // 2
    PW = 2 * DH
    L = M + SEG
    scale_a = DH ** -0.5
    DHB = D // HB
    scale_b = DHB ** -0.5
    NTB = D // 128
    NPRE = CFG['npre']
    XH = (NPRE + 4) * SEG
    WIN = CFG["win"]

    def w_copy(m, p):
        src, dst = ((wk_hbm, lk_ref), (wq_hbm, lq_ref), (wv_hbm, lv_ref), (wo_hbm, lo_ref))[m]
        rows = pl.ds(pl.multiple_of(p * PW, PW), PW)
        return pltpu.make_async_copy(src.at[rows, :], dst.at[rows, :], sem.at[4 * p + m])

    c_xh = pltpu.make_async_copy(x_hbm.at[pl.ds(0, XH), :], x_ref.at[pl.ds(0, XH), :], sem.at[4 * NP])
    c_xr = pltpu.make_async_copy(x_hbm.at[pl.ds(XH, S - XH), :], x_ref.at[pl.ds(XH, S - XH), :], sem.at[4 * NP + 1])
    c_bq = pltpu.make_async_copy(bqkv_hbm, lbqkv_ref, sem.at[4 * NP + 2])
    c_bo = pltpu.make_async_copy(bwo_hbm, lbwo_ref, sem.at[4 * NP + 3])
    S1 = (NSEG - 3) * SEG
    c_o1 = pltpu.make_async_copy(out_ref.at[pl.ds(0, S1), :], out_hbm.at[pl.ds(0, S1), :], sem.at[4 * NP + 4])
    c_o2 = pltpu.make_async_copy(out_ref.at[pl.ds(S1, S - S1), :], out_hbm.at[pl.ds(S1, S - S1), :], sem.at[4 * NP + 5])

    def issue(p):
        for m in (1, 2, 3):
            w_copy(m, p).start()

    c_xh.start()
    w_copy(0, 0).start()
    for p in range(WIN):
        issue(p)
        w_copy(0, p + 1).start()

    r = lax.broadcasted_iota(jnp.int32, (L, 128), 0)
    l = lax.broadcasted_iota(jnp.int32, (L, 128), 1)
    slot = jnp.where(l >= L, l - L, l)
    valid = (l < 2 * L) & ((r < M) | (r >= slot))
    in_h = l < L
    in_g = (l >= L) & (l < 2 * L)
    lo = l < 64
    fill = -1e9 / scale_a
    c_exp = scale_a * LOG2E

    def rows_c(a, c):
        if a.shape[0] == L:
            return a
        return jnp.concatenate([a[M * c:M * c + M], a[2 * M + SEG * c:2 * M + SEG * c + SEG]], axis=0)

    def blk(a, c, pad):
        a = rows_c(a, c)
        a0, a1, a2 = a[:, 0:128], a[:, 128:256], a[:, 256:384]
        z = jnp.zeros((L, 128), F32)
        top = jnp.concatenate([a0, jnp.where(lo, a1, 0.0), z], axis=1)
        bot = jnp.concatenate([z, jnp.where(lo, 0.0, a1), a2], axis=1)
        parts = [top, bot] + ([jnp.zeros((128 - 2 * L, PW), F32)] if pad else [])
        return jnp.concatenate(parts, axis=0).astype(BF16)

    def qk(q, k, chains):
        return [_dot(rows_c(q, c), blk(k, c, False), NT) for c in chains]

    def attn_c(s, v, c):
        s = jnp.concatenate([s, jnp.full((L, 128 - 2 * L), fill, F32)], axis=1)
        s = jnp.where(valid, s, fill)
        mh = jnp.max(jnp.where(in_h, s, -jnp.inf), axis=-1, keepdims=True)
        mg = jnp.max(jnp.where(in_g, s, -jnp.inf), axis=-1, keepdims=True)
        e = jnp.exp2((s - jnp.where(in_h, mh, mg)) * c_exp)
        e = jnp.where(l < 2 * L, e, 0.0)
        ih = _rcp(jnp.sum(jnp.where(in_h, e, 0.0), axis=-1, keepdims=True))
        ig = _rcp(jnp.sum(jnp.where(in_g, e, 0.0), axis=-1, keepdims=True))
        o = _dot(e, blk(v, c, True))
        return jnp.concatenate([o[:, 0:128] * ih, o[:, 128:256] * jnp.where(lo, ih, ig), o[:, 256:384] * ig], axis=1)

    def pv(ss, v, chains):
        os_ = [attn_c(s, v, c) for s, c in zip(ss, chains)]
        if len(chains) == 2:
            return jnp.concatenate([os_[0][0:M], os_[1][0:M], os_[0][M:L], os_[1][M:L]], axis=0)
        return os_[0]

    def seg_rows(s):
        if isinstance(s, int):
            return pl.ds(s * SEG, SEG)
        return pl.ds(pl.multiple_of(s * SEG, SEG), SEG)

    mem0 = mem0_ref[...]
    y_ref[...] = jnp.zeros(y_ref.shape, F32)
    x2_ref[...] = jnp.zeros(x2_ref.shape, F32)
    kb_ref[...] = jnp.zeros(kb_ref.shape, F32)
    vb_ref[...] = jnp.zeros(vb_ref.shape, F32)
    acc0_ref[...] = jnp.zeros(acc0_ref.shape, F32)
    c_xh.wait()
    h0_ref[0:M, :] = mem0.astype(F32)
    h0_ref[M:L, :] = _ln(x_ref[0:SEG, :].astype(F32)).astype(BF16).astype(F32)
    h0_ref[L:L + NPRE * SEG, :] = _ln(x_ref[2 * SEG:(2 + NPRE) * SEG, :].astype(F32)).astype(BF16).astype(F32)


    def conv_body(p, carry):
        for m in (1, 2, 3):
            w_copy(m, p).wait()

        @pl.when(p + 1 < NP)
        def _():
            w_copy(0, p + 1).wait()

        @pl.when(p + WIN < NP)
        def _():
            issue(p + WIN)

        @pl.when(p + WIN + 1 < NP)
        def _():
            w_copy(0, p + WIN + 1).start()

        @pl.when(p + WIN == NP)
        def _():
            c_bq.start()
            c_bo.start()
            c_xr.start()

        rows = pl.ds(pl.multiple_of(p * PW, PW), PW)
        pp = jnp.maximum(p - 1, 0)
        ss = qk(qp_ref[pp, 0:L, :], kp_ref[pp, 0:L, :], (0,))
        vprev = vp_ref[pp, 0:L, :]
        woprev = _unpack(wo_ref[pp])
        h = h0_ref[...]
        k = _dot(h, _unpack(wk_ref[p]))
        wq = lq_ref[rows, :].T
        wq_ref[p] = _pack(wq)
        q = _dot(h, wq)
        o = pv(ss, vprev, (0,))
        wv = lv_ref[rows, :].T
        wv_ref[p] = _pack(wv)
        v = _dot(h, wv)
        acc0_ref[...] += _dot(o, woprev)
        wo_ref[p] = _pack(lo_ref[rows, :])
        pn = jnp.minimum(p + 1, NP - 1)
        wk_ref[pn] = _pack(lk_ref[pl.ds(pl.multiple_of(pn * PW, PW), PW), :].T)
        kp_ref[p] = k
        qp_ref[p] = q
        vp_ref[p] = v
        return carry

    def b_perm_in(j):
        if j == 0:
            c_bq.wait()
            c_bo.wait()
        for c in range(NTB):
            for i in range(NTB):
                if j < 3:
                    t_ = lbqkv_ref[c * 128:(c + 1) * 128, j * D + i * 128:j * D + (i + 1) * 128].T
                else:
                    t_ = lbwo_ref[i * 128:(i + 1) * 128, c * 128:(c + 1) * 128]
                tf_ref[j, c, i * 128:(i + 1) * 128, :] = t_.astype(F32)

    def b_perm_out(j):
        for c in range(NTB):
            for g in range(NTB):
                t_ = jnp.concatenate([tf_ref[j, c, pl.ds(d, HB, stride=DHB), :]
                                      for d in range(4 * g, 4 * g + 4)], axis=0).astype(BF16)
                if j < 3:
                    bqkvp_ref[c * 64:(c + 1) * 64, j * D + g * 128:j * D + (g + 1) * 128] = _pack(t_.T)
                else:
                    bwop_ref[g * 64:(g + 1) * 64, c * 128:(c + 1) * 128] = _pack(t_)

    def b_perm(p):
        if 0 <= p < 4:
            b_perm_in(p)
        if 1 <= p < 5:
            b_perm_out(p - 1)

    w_copy(0, 0).wait()
    wk_ref[0] = _pack(lk_ref[0:PW, :].T)
    for r_ in (qp_ref, kp_ref, vp_ref):
        r_[0, 0:L, :] = jnp.zeros((L, PW), F32)
    wo_ref[0] = jnp.zeros(wo_ref.shape[1:], U32)
    lax.fori_loop(0, NP, conv_body, 0)
    o_ = pv(qk(qp_ref[NP - 1, 0:L, :], kp_ref[NP - 1, 0:L, :], (0,)), vp_ref[NP - 1, 0:L, :], (0,))
    acc0_ref[...] += _dot(o_, _unpack(wo_ref[NP - 1]))
    acc0 = acc0_ref[...]
    h_ref[0:2 * M, :] = jnp.concatenate([acc0[0:M], mem0.astype(F32)], axis=0).astype(BF16)
    h_ref[2 * M:2 * M + SEG, :] = _ln(x_ref[seg_rows(1), :].astype(F32)).astype(BF16)
    h_ref[2 * M + SEG:2 * L, :] = jnp.zeros((SEG, D), BF16)
    y_ref[0:SEG, :] = x_ref[seg_rows(0), :].astype(F32) + acc0[M:L]

    rowi = lax.broadcasted_iota(jnp.int32, (16, 128), 0)
    fill_b = -1e9 / scale_b
    c_expb = scale_b * LOG2E

    def b_front():
        qkv = _dot(_ln(y_ref[...]).astype(BF16), _unpack(bqkvp_ref[...]))
        for lyr in range(2):
            for j in range(NTB):
                kb_ref[lyr, j, 16:48, :] = qkv[32 * lyr:32 * lyr + 32, D + 128 * j:D + 128 * j + 128]
                vb_ref[lyr, j, 16:48, :] = qkv[32 * lyr:32 * lyr + 32, 2 * D + 128 * j:2 * D + 128 * j + 128]
        return qkv[:, 0:D]

    def b_attn(q, t, lyr):
        seg = t - 1 - 2 * lyr
        q = q[32 * lyr:32 * lyr + 32]
        logits = []
        for w in range(W):
            tt = None
            for j in range(NTB):
                pr = q[:, 128 * j:128 * j + 128] * kb_ref[lyr, j, 16 - DIL * w:48 - DIL * w, :]
                tt = pr if tt is None else tt + pr
            tt = tt + pltpu.roll(tt, 64, 1)
            tt = tt + pltpu.roll(tt, 32, 1)
            if w > 0:
                top = jnp.where(rowi >= DIL * w - seg * SEG, tt[0:16], fill_b)
                tt = jnp.concatenate([top, tt[16:32]], axis=0)
            logits.append(tt)
        mx = functools.reduce(jnp.maximum, logits)
        es = [jnp.exp2((t_ - mx) * c_expb) for t_ in logits]
        inv = _rcp(functools.reduce(lambda a, b: a + b, es))
        outs = []
        for j in range(NTB):
            o = None
            for w in range(W):
                c = es[w] * vb_ref[lyr, j, 16 - DIL * w:48 - DIL * w, :]
                o = c if o is None else o + c
            outs.append(o * inv)
        for j in range(NTB):
            kb_ref[lyr, j, 0:16, :] = kb_ref[lyr, j, 32:48, :]
            vb_ref[lyr, j, 0:16, :] = vb_ref[lyr, j, 32:48, :]
        return jnp.concatenate(outs, axis=1)

    def b_back(o, lyr):
        return y_ref[32 * lyr:32 * lyr + 32, :] + _dot(o, _unpack(bwop_ref[...]))

    def step(t, chains, pre=False, hook=None, bf=CFG['bf'], wo0=CFG['wo0']):
        dual = len(chains) == 2
        if pre:
            h = jnp.concatenate([h_ref[0:2 * M, :], h_ref[2 * M + SEG:2 * L, :]], axis=0)
        elif dual:
            h = h_ref[...]
        else:
            h = rows_c(h_ref[...].astype(F32), chains[0])
        x2_res = x2_ref[...] if 1 in chains else None
        st = {}

        def b0():
            z = b_back(b_attn(st["q"], t, 0), 0)
            x2_ref[...] = z
            h_ref[2 * M + SEG:2 * L, :] = _ln(z).astype(BF16)

        def b1():
            z = b_back(b_attn(st["q"], t, 1), 1)
            out_ref[seg_rows(jnp.maximum(t - 3, 0)), :] = z.astype(out_ref.dtype)

        def prj(w_ref, p, cols=slice(None)):
            r_ = _dot(h, _unpack(w_ref[p, :, cols]))
            if pre:
                p_ref = kp_ref if w_ref is wk_ref else (qp_ref if w_ref is wq_ref else vp_ref)
                xs = p_ref[p, pl.ds(pl.multiple_of(L + (t - 2) * SEG, 8), SEG), cols]
                r_ = jnp.concatenate([r_[0:2 * M], xs, r_[2 * M:L + M]], axis=0)
            return r_

        def opj(o, p):
            return _dot(o, _unpack(wo_ref[p]))

        k = prj(wk_ref, 0)
        q = prj(wq_ref, 0)
        v = prj(wv_ref, 0)
        acc = None
        for p in range(NP):
            ss = qk(q, k, chains)
            if hook is not None:
                hook(p)
            if p == bf:
                st["q"] = b_front()
            if p == CFG["lnx"] and 0 in chains:
                tn = min(t + 1, NSEG - 1) if isinstance(t, int) else jnp.minimum(t + 1, NSEG - 1)
                h_ref[2 * M:2 * M + SEG, :] = _ln(x_ref[seg_rows(tn), :].astype(F32)).astype(BF16)
            if p + 1 < NP:
                q = prj(wq_ref, p + 1)
                k = prj(wk_ref, p + 1)
            else:
                if CFG["vsplit"]:
                    v = jnp.concatenate([v, prj(wv_ref, p, slice(256, 384))], axis=1)
                acc = acc + opj(o, p - 1)
            o = pv(ss, v, chains)
            if p + 2 < NP:
                v = prj(wv_ref, p + 1)
            elif p + 2 == NP:
                v = prj(wv_ref, p + 1, slice(0, 256)) if CFG["vsplit"] else prj(wv_ref, p + 1)
            elif 1 in chains:
                b1()
            if p != NP - 2:
                d = opj(o, p)
                acc = d if acc is None else acc + d
            if p == wo0:
                b0()

        if dual:
            h_ref[0:2 * M, :] = acc[0:2 * M].astype(BF16)
            y_ref[0:SEG, :] = x_ref[seg_rows(t), :].astype(F32) + acc[2 * M:2 * M + SEG]
            y_ref[SEG:2 * SEG, :] = x2_res + acc[2 * M + SEG:2 * L]
        elif chains[0] == 0:
            h_ref[0:M, :] = acc[0:M].astype(BF16)
            y_ref[0:SEG, :] = x_ref[seg_rows(t), :].astype(F32) + acc[M:L]
        else:
            h_ref[M:2 * M, :] = acc[0:M].astype(BF16)
            y_ref[SEG:2 * SEG, :] = x2_res + acc[M:L]

    def run(lo_, hi_, chains, pre=False):
        def body(t, carry):
            step(t, chains, pre)
            return carry
        lax.fori_loop(lo_, hi_, body, 0)

    PB = CFG["pb"]
    step(1, (0,), hook=lambda p: b_perm(p - PB), bf=PB + 6, wo0=PB + 9)
    c_xr.wait()
    if NPRE:
        run(2, 2 + NPRE, (0, 1), True)
    run(2 + NPRE, 2 + CFG["nit"], (0, 1))
    c_o1.start()
    run(NSEG, NSEG + 2, (1,))
    z = b_back(b_attn(b_front(), NSEG + 2, 1), 1)
    out_ref[seg_rows(NSEG - 1), :] = z.astype(out_ref.dtype)
    c_o2.start()
    c_o1.wait()
    c_o2.wait()


@functools.partial(jax.jit, static_argnames=("A_seg_len",))
def pallas_interleave_layers__memory_aug_recurrent_mem_tr__sliding_local_dilated__prompt_kernel(
    A_x, A_mem0, A_Wq, A_Wk, A_Wv, A_Wo, A_seg_len, B_x, B_wqkv, B_wo,
):
    del B_x
    B, S, D = A_x.shape
    _, H, DH = A_Wq.shape
    M = A_mem0.shape[1]
    SEG = int(A_seg_len)
    assert B == 1 and M == 8 and SEG == 32 and DH == 192 and D == 640
    NP, PW = H // 2, 2 * DH

    x = A_x.reshape(S, D)
    mem0 = A_mem0.reshape(M, D)
    wq = A_Wq.transpose(1, 2, 0).reshape(H * DH, D)
    wk = A_Wk.transpose(1, 2, 0).reshape(H * DH, D)
    wv = A_Wv.transpose(1, 2, 0).reshape(H * DH, D)
    wo = A_Wo.reshape(H * DH, D)

    kern = functools.partial(_kernel, S=S, D=D, H=H, DH=DH, M=M, SEG=SEG, HB=32, W=8, DIL=2)
    hbm = pl.BlockSpec(memory_space=pl.ANY)
    out = pl.pallas_call(
        kern,
        out_shape=jax.ShapeDtypeStruct((S, D), A_x.dtype),
        in_specs=[hbm, pl.BlockSpec(memory_space=pltpu.VMEM), hbm, hbm, hbm, hbm, hbm, hbm],
        out_specs=hbm,
        scratch_shapes=[
            pltpu.VMEM((S, D), BF16),
            pltpu.VMEM((S, D), A_x.dtype),
            pltpu.VMEM((H * DH, D), BF16),
            pltpu.VMEM((H * DH, D), BF16),
            pltpu.VMEM((H * DH, D), BF16),
            pltpu.VMEM((H * DH, D), BF16),
            pltpu.VMEM((NP, D // 2, PW), U32),
            pltpu.VMEM((NP, D // 2, PW), U32),
            pltpu.VMEM((NP, D // 2, PW), U32),
            pltpu.VMEM((NP, PW // 2, D), U32),
            pltpu.VMEM((D, 3 * D), BF16),
            pltpu.VMEM((D, D), BF16),
            pltpu.VMEM((4, D // 128, D, 128), F32),
            pltpu.VMEM((D // 2, 3 * D), U32),
            pltpu.VMEM((D // 2, D), U32),
            pltpu.VMEM((2 * (M + SEG), D), BF16),
            pltpu.VMEM((2 * SEG, D), F32),
            pltpu.VMEM((SEG, D), F32),
            pltpu.VMEM((2, D // 128, 48, 128), F32),
            pltpu.VMEM((2, D // 128, 48, 128), F32),
            pltpu.VMEM((M + SEG + CFG["npre"] * SEG, D), F32),
            pltpu.VMEM((M + SEG, D), F32),
            pltpu.VMEM((NP, M + SEG + CFG["npre"] * SEG, PW), F32),
            pltpu.VMEM((NP, M + SEG + CFG["npre"] * SEG, PW), F32),
            pltpu.VMEM((NP, M + SEG + CFG["npre"] * SEG, PW), F32),
            pltpu.SemaphoreType.DMA((4 * NP + 6,)),
        ],
        compiler_params=pltpu.CompilerParams(vmem_limit_bytes=110 * 1024 * 1024),
    )(x, mem0, wq, wk, wv, wo, B_wqkv, B_wo)
    return out.reshape(B, S, D)
```

```python
import functools

import jax
import jax.numpy as jnp
from jax import lax
import jax.experimental.pallas as pl
import jax.experimental.pallas.tpu as pltpu

F32 = jnp.float32
BF16 = jnp.bfloat16
U32 = jnp.uint32
NT = (((1,), (1,)), ((), ()))
NN = (((1,), (0,)), ((), ()))
LOG2E = 1.4426950408889634

CFG = dict(wo0=10, bf=0, lnx=9, win=4, nit=62, vsplit=1, npre=8, pb=2, wo1=14, bf1=8, ob16=1)


def _ln(x):
    m = jnp.mean(x, axis=-1, keepdims=True)
    xc = x - m
    v = jnp.mean(xc * xc, axis=-1, keepdims=True)
    return xc * lax.rsqrt(v + 1e-5)


def _dot(a, b, dims=NN):
    return lax.dot_general(a, b, dims, preferred_element_type=F32)


def _rcp(x):
    r_ = pl.reciprocal(x, approx=True)
    return r_ * (2.0 - x * r_)


def _pack(x):
    return pltpu.bitcast(x, U32)


def _unpack(x):
    return pltpu.bitcast(x, BF16)


def _kernel(x_hbm, mem0_ref, wq_hbm, wk_hbm, wv_hbm, wo_hbm, bqkv_hbm, bwo_hbm,
            out_hbm,
            x_ref, out_ref, lq_ref, lk_ref, lv_ref, lo_ref, wq_ref, wk_ref, wv_ref, wo_ref,
            lbqkv_ref, lbwo_ref, tf_ref, bqkvp_ref, bwop_ref,
            h_ref, y_ref, x2_ref, kb_ref, vb_ref, h0_ref, acc0_ref, qp_ref, kp_ref, vp_ref, sem,
            *, S, D, H, DH, M, SEG, HB, W, DIL):
    NSEG = S // SEG
    NP = H // 2
    PW = 2 * DH
    L = M + SEG
    scale_a = DH ** -0.5
    DHB = D // HB
    scale_b = DHB ** -0.5
    NTB = D // 128
    NPRE = CFG['npre']
    XH = (NPRE + 4) * SEG
    WIN = CFG["win"]

    def w_copy(m, p):
        src, dst = ((wk_hbm, lk_ref), (wq_hbm, lq_ref), (wv_hbm, lv_ref), (wo_hbm, lo_ref))[m]
        rows = pl.ds(pl.multiple_of(p * PW, PW), PW)
        return pltpu.make_async_copy(src.at[rows, :], dst.at[rows, :], sem.at[4 * p + m])

    c_xh = pltpu.make_async_copy(x_hbm.at[pl.ds(0, XH), :], x_ref.at[pl.ds(0, XH), :], sem.at[4 * NP])
    c_xr = pltpu.make_async_copy(x_hbm.at[pl.ds(XH, S - XH), :], x_ref.at[pl.ds(XH, S - XH), :], sem.at[4 * NP + 1])
    c_bq = pltpu.make_async_copy(bqkv_hbm, lbqkv_ref, sem.at[4 * NP + 2])
    c_bo = pltpu.make_async_copy(bwo_hbm, lbwo_ref, sem.at[4 * NP + 3])
    S1 = (NSEG - 3) * SEG
    c_o1 = pltpu.make_async_copy(out_ref.at[pl.ds(0, S1), :], out_hbm.at[pl.ds(0, S1), :], sem.at[4 * NP + 4])
    c_o2 = pltpu.make_async_copy(out_ref.at[pl.ds(S1, S - S1), :], out_hbm.at[pl.ds(S1, S - S1), :], sem.at[4 * NP + 5])

    def issue(p):
        for m in (1, 2, 3):
            w_copy(m, p).start()

    c_xh.start()
    w_copy(0, 0).start()
    for p in range(WIN):
        issue(p)
        w_copy(0, p + 1).start()

    r = lax.broadcasted_iota(jnp.int32, (L, 128), 0)
    l = lax.broadcasted_iota(jnp.int32, (L, 128), 1)
    slot = jnp.where(l >= L, l - L, l)
    valid = (l < 2 * L) & ((r < M) | (r >= slot))
    in_h = l < L
    in_g = (l >= L) & (l < 2 * L)
    lo = l < 64
    fill = -1e9 / scale_a
    c_exp = scale_a * LOG2E

    def rows_c(a, c):
        if a.shape[0] == L:
            return a
        return jnp.concatenate([a[M * c:M * c + M], a[2 * M + SEG * c:2 * M + SEG * c + SEG]], axis=0)

    def blk(a, c, pad):
        a = rows_c(a, c)
        a0, a1, a2 = a[:, 0:128], a[:, 128:256], a[:, 256:384]
        z = jnp.zeros((L, 128), F32)
        top = jnp.concatenate([a0, jnp.where(lo, a1, 0.0), z], axis=1)
        bot = jnp.concatenate([z, jnp.where(lo, 0.0, a1), a2], axis=1)
        parts = [top, bot] + ([jnp.zeros((128 - 2 * L, PW), F32)] if pad else [])
        return jnp.concatenate(parts, axis=0).astype(BF16)

    def qk(q, k, chains):
        return [_dot(rows_c(q, c), blk(k, c, False), NT) for c in chains]

    def attn_c(s, v, c):
        s = jnp.concatenate([s, jnp.full((L, 128 - 2 * L), fill, F32)], axis=1)
        s = jnp.where(valid, s, fill)
        mh = jnp.max(jnp.where(in_h, s, -jnp.inf), axis=-1, keepdims=True)
        mg = jnp.max(jnp.where(in_g, s, -jnp.inf), axis=-1, keepdims=True)
        e = jnp.exp2((s - jnp.where(in_h, mh, mg)) * c_exp)
        e = jnp.where(l < 2 * L, e, 0.0)
        ih = _rcp(jnp.sum(jnp.where(in_h, e, 0.0), axis=-1, keepdims=True))
        ig = _rcp(jnp.sum(jnp.where(in_g, e, 0.0), axis=-1, keepdims=True))
        o = _dot(e, blk(v, c, True))
        return jnp.concatenate([o[:, 0:128] * ih, o[:, 128:256] * jnp.where(lo, ih, ig), o[:, 256:384] * ig], axis=1)

    def pv(ss, v, chains):
        os_ = [attn_c(s, v, c) for s, c in zip(ss, chains)]
        if len(chains) == 2:
            return jnp.concatenate([os_[0][0:M], os_[1][0:M], os_[0][M:L], os_[1][M:L]], axis=0)
        return os_[0]

    def seg_rows(s):
        if isinstance(s, int):
            return pl.ds(s * SEG, SEG)
        return pl.ds(pl.multiple_of(s * SEG, SEG), SEG)

    mem0 = mem0_ref[...]
    y_ref[...] = jnp.zeros(y_ref.shape, F32)
    x2_ref[...] = jnp.zeros(x2_ref.shape, F32)
    kb_ref[...] = jnp.zeros(kb_ref.shape, F32)
    vb_ref[...] = jnp.zeros(vb_ref.shape, F32)
    acc0_ref[...] = jnp.zeros(acc0_ref.shape, F32)
    c_xh.wait()
    h0_ref[0:M, :] = mem0.astype(F32)
    h0_ref[M:L, :] = _ln(x_ref[0:SEG, :].astype(F32)).astype(BF16).astype(F32)
    h0_ref[L:L + NPRE * SEG, :] = _ln(x_ref[2 * SEG:(2 + NPRE) * SEG, :].astype(F32)).astype(BF16).astype(F32)


    def conv_body(p, carry):
        for m in (1, 2, 3):
            w_copy(m, p).wait()

        @pl.when(p + 1 < NP)
        def _():
            w_copy(0, p + 1).wait()

        @pl.when(p + WIN < NP)
        def _():
            issue(p + WIN)

        @pl.when(p + WIN + 1 < NP)
        def _():
            w_copy(0, p + WIN + 1).start()

        @pl.when(p + WIN == NP)
        def _():
            c_bq.start()
            c_bo.start()
            c_xr.start()

        rows = pl.ds(pl.multiple_of(p * PW, PW), PW)
        pp = jnp.maximum(p - 1, 0)
        ss = qk(qp_ref[pp, 0:L, :], kp_ref[pp, 0:L, :], (0,))
        vprev = vp_ref[pp, 0:L, :]
        woprev = _unpack(wo_ref[pp])
        h = h0_ref[...]
        k = _dot(h, _unpack(wk_ref[p]))
        wq = lq_ref[rows, :].T
        wq_ref[p] = _pack(wq)
        q = _dot(h, wq)
        o = pv(ss, vprev, (0,))
        wv = lv_ref[rows, :].T
        wv_ref[p] = _pack(wv)
        v = _dot(h, wv)
        acc0_ref[...] += _dot(o, woprev)
        wo_ref[p] = _pack(lo_ref[rows, :])
        pn = jnp.minimum(p + 1, NP - 1)
        wk_ref[pn] = _pack(lk_ref[pl.ds(pl.multiple_of(pn * PW, PW), PW), :].T)
        kp_ref[p] = k
        qp_ref[p] = q
        vp_ref[p] = v
        return carry

    def b_perm_in(j):
        for c in range(NTB):
            if j < 3:
                t_ = lbqkv_ref[c * 128:(c + 1) * 128, j * D:(j + 1) * D].T
            else:
                t_ = lbwo_ref[:, c * 128:(c + 1) * 128]
            tf_ref[j, c] = t_.astype(F32)

    def b_perm_out(j):
        for c in range(NTB):
            t_ = jnp.concatenate([tf_ref[j, c, pl.ds(d, HB, stride=DHB), :] for d in range(DHB)], axis=0)
            t_ = t_.astype(BF16)
            if j < 3:
                bqkvp_ref[c * 64:(c + 1) * 64, j * D:(j + 1) * D] = _pack(t_.T)
            else:
                bwop_ref[:, c * 128:(c + 1) * 128] = _pack(t_)

    w_copy(0, 0).wait()
    wk_ref[0] = _pack(lk_ref[0:PW, :].T)
    for r_ in (qp_ref, kp_ref, vp_ref):
        r_[0, 0:L, :] = jnp.zeros((L, PW), F32)
    wo_ref[0] = jnp.zeros(wo_ref.shape[1:], U32)
    lax.fori_loop(0, NP, conv_body, 0)
    o_ = pv(qk(qp_ref[NP - 1, 0:L, :], kp_ref[NP - 1, 0:L, :], (0,)), vp_ref[NP - 1, 0:L, :], (0,))
    acc0_ref[...] += _dot(o_, _unpack(wo_ref[NP - 1]))
    acc0 = acc0_ref[...]
    h_ref[0:2 * M, :] = jnp.concatenate([acc0[0:M], mem0.astype(F32)], axis=0).astype(BF16)
    h_ref[2 * M:2 * M + SEG, :] = _ln(x_ref[seg_rows(1), :].astype(F32)).astype(BF16)
    h_ref[2 * M + SEG:2 * L, :] = jnp.zeros((SEG, D), BF16)
    y_ref[0:SEG, :] = x_ref[seg_rows(0), :].astype(F32) + acc0[M:L]

    rowi = lax.broadcasted_iota(jnp.int32, (16, 128), 0)
    fill_b = -1e9 / scale_b
    c_expb = scale_b * LOG2E

    def b_front(lyrs=(0, 1), js=(0, 1, 2), hb=None):
        r0, r1 = SEG * lyrs[0], SEG * lyrs[-1] + SEG
        if hb is None:
            hb = _ln(y_ref[r0:r1, :]).astype(BF16)
        qkv = _dot(hb, _unpack(bqkvp_ref[:, js[0] * D:(js[-1] + 1) * D]))
        for n, j in enumerate(js):
            if j == 0:
                continue
            dst = kb_ref if j == 1 else vb_ref
            for lyr in lyrs:
                for c in range(NTB):
                    dst[lyr, c, 16:48, :] = qkv[SEG * lyr - r0:SEG * lyr - r0 + SEG, n * D + 128 * c:n * D + 128 * c + 128]
        return (qkv[:, 0:D] if js[0] == 0 else None), hb

    def b_attn(q, t, lyr):
        seg = t - 1 - 2 * lyr
        if q.shape[0] != SEG:
            q = q[SEG * lyr:SEG * lyr + SEG]
        logits = []
        for w in range(W):
            tt = None
            for j in range(NTB):
                pr = q[:, 128 * j:128 * j + 128] * kb_ref[lyr, j, 16 - DIL * w:48 - DIL * w, :]
                tt = pr if tt is None else tt + pr
            tt = tt + pltpu.roll(tt, 64, 1)
            tt = tt + pltpu.roll(tt, 32, 1)
            if w > 0:
                top = jnp.where(rowi >= DIL * w - seg * SEG, tt[0:16], fill_b)
                tt = jnp.concatenate([top, tt[16:32]], axis=0)
            logits.append(tt)
        mx = functools.reduce(jnp.maximum, logits)
        es = [jnp.exp2((t_ - mx) * c_expb) for t_ in logits]
        inv = _rcp(functools.reduce(lambda a, b: a + b, es))
        outs = []
        for j in range(NTB):
            o = None
            for w in range(W):
                c = es[w] * vb_ref[lyr, j, 16 - DIL * w:48 - DIL * w, :]
                o = c if o is None else o + c
            outs.append(o * inv)
        for j in range(NTB):
            kb_ref[lyr, j, 0:16, :] = kb_ref[lyr, j, 32:48, :]
            vb_ref[lyr, j, 0:16, :] = vb_ref[lyr, j, 32:48, :]
        return jnp.concatenate(outs, axis=1)

    def b_back(o, lyr):
        return y_ref[32 * lyr:32 * lyr + 32, :] + _dot(o, _unpack(bwop_ref[...]))

    def step(t, chains, pre=False, hook=None, bf=CFG['bf'], wo0=CFG['wo0']):
        dual = len(chains) == 2
        if pre:
            h = jnp.concatenate([h_ref[0:2 * M, :], h_ref[2 * M + SEG:2 * L, :]], axis=0)
        elif dual:
            h = h_ref[...]
        else:
            h = rows_c(h_ref[...].astype(F32), chains[0])
        x2_res = x2_ref[...] if 1 in chains else None
        st = {}

        def b0():
            z = b_back(b_attn(st["q"], t, 0), 0)
            x2_ref[...] = z
            h_ref[2 * M + SEG:2 * L, :] = _ln(z).astype(BF16)

        def b1():
            z = b_back(b_attn(st["q"], t, 1), 1)
            out_ref[seg_rows(jnp.maximum(t - 3, 0)), :] = z.astype(out_ref.dtype)

        def prj(w_ref, p, cols=slice(None)):
            r_ = _dot(h, _unpack(w_ref[p, :, cols]))
            if pre:
                p_ref = kp_ref if w_ref is wk_ref else (qp_ref if w_ref is wq_ref else vp_ref)
                xs = p_ref[p, pl.ds(pl.multiple_of(L + (t - 2) * SEG, 8), SEG), cols]
                r_ = jnp.concatenate([r_[0:2 * M], xs, r_[2 * M:L + M]], axis=0)
            return r_

        def opj(o, p):
            if CFG["ob16"] and dual:
                o = o.astype(BF16)
            return _dot(o, _unpack(wo_ref[p]))

        k = prj(wk_ref, 0)
        q = prj(wq_ref, 0)
        v = prj(wv_ref, 0)
        acc = None
        for p in range(NP):
            ss = qk(q, k, chains)
            if hook is not None:
                hook(p, st)
            if hook is None and p == bf:
                st["q"] = b_front()[0]
            if p == CFG["lnx"] and 0 in chains:
                tn = min(t + 1, NSEG - 1) if isinstance(t, int) else jnp.minimum(t + 1, NSEG - 1)
                h_ref[2 * M:2 * M + SEG, :] = _ln(x_ref[seg_rows(tn), :].astype(F32)).astype(BF16)
            if p + 1 < NP:
                q = prj(wq_ref, p + 1)
                k = prj(wk_ref, p + 1)
            else:
                if CFG["vsplit"]:
                    v = jnp.concatenate([v, prj(wv_ref, p, slice(256, 384))], axis=1)
                acc = acc + opj(o, p - 1)
            o = pv(ss, v, chains)
            if p + 2 < NP:
                v = prj(wv_ref, p + 1)
            elif p + 2 == NP:
                v = prj(wv_ref, p + 1, slice(0, 256)) if CFG["vsplit"] else prj(wv_ref, p + 1)
            elif 1 in chains:
                b1()
            if p != NP - 2:
                d = opj(o, p)
                acc = d if acc is None else acc + d
            if p == wo0:
                b0()

        if dual:
            h_ref[0:2 * M, :] = acc[0:2 * M].astype(BF16)
            y_ref[0:SEG, :] = x_ref[seg_rows(t), :].astype(F32) + acc[2 * M:2 * M + SEG]
            y_ref[SEG:2 * SEG, :] = x2_res + acc[2 * M + SEG:2 * L]
        elif chains[0] == 0:
            h_ref[0:M, :] = acc[0:M].astype(BF16)
            y_ref[0:SEG, :] = x_ref[seg_rows(t), :].astype(F32) + acc[M:L]
        else:
            h_ref[M:2 * M, :] = acc[0:M].astype(BF16)
            y_ref[SEG:2 * SEG, :] = x2_res + acc[M:L]

    def run(lo_, hi_, chains, pre=False):
        def body(t, carry):
            step(t, chains, pre)
            return carry
        lax.fori_loop(lo_, hi_, body, 0)

    PB = CFG["pb"]

    def hook1(p, st):
        if p == PB:
            c_bq.wait()
            c_bo.wait()
        if PB <= p < PB + 4:
            b_perm_in(p - PB)
        if PB + 1 <= p < PB + 5:
            b_perm_out(p - PB - 1)
        if p == PB + CFG["bf1"]:
            st["q"] = b_front((0,))[0]

    step(1, (0,), hook=hook1, wo0=CFG["wo1"])
    c_xr.wait()
    if NPRE:
        run(2, 2 + NPRE, (0, 1), True)
    run(2 + NPRE, 2 + CFG["nit"], (0, 1))
    c_o1.start()
    run(NSEG, NSEG + 2, (1,))
    z = b_back(b_attn(b_front((1,))[0], NSEG + 2, 1), 1)
    out_ref[seg_rows(NSEG - 1), :] = z.astype(out_ref.dtype)
    c_o2.start()
    c_o1.wait()
    c_o2.wait()


@functools.partial(jax.jit, static_argnames=("A_seg_len",))
def pallas_interleave_layers__memory_aug_recurrent_mem_tr__sliding_local_dilated__prompt_kernel(
    A_x, A_mem0, A_Wq, A_Wk, A_Wv, A_Wo, A_seg_len, B_x, B_wqkv, B_wo,
):
    del B_x
    B, S, D = A_x.shape
    _, H, DH = A_Wq.shape
    M = A_mem0.shape[1]
    SEG = int(A_seg_len)
    assert B == 1 and M == 8 and SEG == 32 and DH == 192 and D == 640
    NP, PW = H // 2, 2 * DH

    x = A_x.reshape(S, D)
    mem0 = A_mem0.reshape(M, D)
    wq = A_Wq.transpose(1, 2, 0).reshape(H * DH, D)
    wk = A_Wk.transpose(1, 2, 0).reshape(H * DH, D)
    wv = A_Wv.transpose(1, 2, 0).reshape(H * DH, D)
    wo = A_Wo.reshape(H * DH, D)

    kern = functools.partial(_kernel, S=S, D=D, H=H, DH=DH, M=M, SEG=SEG, HB=32, W=8, DIL=2)
    hbm = pl.BlockSpec(memory_space=pl.ANY)
    out = pl.pallas_call(
        kern,
        out_shape=jax.ShapeDtypeStruct((S, D), A_x.dtype),
        in_specs=[hbm, pl.BlockSpec(memory_space=pltpu.VMEM), hbm, hbm, hbm, hbm, hbm, hbm],
        out_specs=hbm,
        scratch_shapes=[
            pltpu.VMEM((S, D), BF16),
            pltpu.VMEM((S, D), A_x.dtype),
            pltpu.VMEM((H * DH, D), BF16),
            pltpu.VMEM((H * DH, D), BF16),
            pltpu.VMEM((H * DH, D), BF16),
            pltpu.VMEM((H * DH, D), BF16),
            pltpu.VMEM((NP, D // 2, PW), U32),
            pltpu.VMEM((NP, D // 2, PW), U32),
            pltpu.VMEM((NP, D // 2, PW), U32),
            pltpu.VMEM((NP, PW // 2, D), U32),
            pltpu.VMEM((D, 3 * D), BF16),
            pltpu.VMEM((D, D), BF16),
            pltpu.VMEM((4, D // 128, D, 128), F32),
            pltpu.VMEM((D // 2, 3 * D), U32),
            pltpu.VMEM((D // 2, D), U32),
            pltpu.VMEM((2 * (M + SEG), D), BF16),
            pltpu.VMEM((2 * SEG, D), F32),
            pltpu.VMEM((SEG, D), F32),
            pltpu.VMEM((2, D // 128, 48, 128), F32),
            pltpu.VMEM((2, D // 128, 48, 128), F32),
            pltpu.VMEM((M + SEG + CFG["npre"] * SEG, D), F32),
            pltpu.VMEM((M + SEG, D), F32),
            pltpu.VMEM((NP, M + SEG + CFG["npre"] * SEG, PW), F32),
            pltpu.VMEM((NP, M + SEG + CFG["npre"] * SEG, PW), F32),
            pltpu.VMEM((NP, M + SEG + CFG["npre"] * SEG, PW), F32),
            pltpu.SemaphoreType.DMA((4 * NP + 6,)),
        ],
        compiler_params=pltpu.CompilerParams(vmem_limit_bytes=110 * 1024 * 1024),
    )(x, mem0, wq, wk, wv, wo, B_wqkv, B_wo)
    return out.reshape(B, S, D)
```

```python
import functools

import jax
import jax.numpy as jnp
from jax import lax
import jax.experimental.pallas as pl
import jax.experimental.pallas.tpu as pltpu

F32 = jnp.float32
BF16 = jnp.bfloat16
U32 = jnp.uint32
NT = (((1,), (1,)), ((), ()))
NN = (((1,), (0,)), ((), ()))
LOG2E = 1.4426950408889634

NPRE = 8
DMA_WIN = 4
P_BFRONT, P_LNX, P_B0 = 0, 9, 10
P1_PERM, P1_BFRONT, P1_B0 = 2, 10, 14


def _ln(x):
    m = jnp.mean(x, axis=-1, keepdims=True)
    xc = x - m
    v = jnp.mean(xc * xc, axis=-1, keepdims=True)
    return xc * lax.rsqrt(v + 1e-5)


def _dot(a, b, dims=NN):
    return lax.dot_general(a, b, dims, preferred_element_type=F32)


def _rcp(x):
    r = pl.reciprocal(x, approx=True)
    return r * (2.0 - x * r)


def _pack(x):
    return pltpu.bitcast(x, U32)


def _unpack(x):
    return pltpu.bitcast(x, BF16)


def _kernel(x_hbm, mem0_ref, wq_hbm, wk_hbm, wv_hbm, wo_hbm, bqkv_hbm, bwo_hbm,
            out_hbm,
            x_ref, out_ref, lq_ref, lk_ref, lv_ref, lo_ref, wq_ref, wk_ref, wv_ref, wo_ref,
            lbqkv_ref, lbwo_ref, tf_ref, bqkvp_ref, bwop_ref,
            h_ref, y_ref, x2_ref, kb_ref, vb_ref, h0_ref, acc0_ref, qp_ref, kp_ref, vp_ref, sem,
            *, S, D, H, DH, M, SEG, HB, W, DIL):
    NSEG = S // SEG
    NP = H // 2
    PW = 2 * DH
    L = M + SEG
    scale_a = DH ** -0.5
    DHB = D // HB
    scale_b = DHB ** -0.5
    NTB = D // 128
    HIST = DIL * W
    XH = (NPRE + 4) * SEG

    def w_copy(m, p):
        src, dst = ((wk_hbm, lk_ref), (wq_hbm, lq_ref), (wv_hbm, lv_ref), (wo_hbm, lo_ref))[m]
        rows = pl.ds(pl.multiple_of(p * PW, PW), PW)
        return pltpu.make_async_copy(src.at[rows, :], dst.at[rows, :], sem.at[4 * p + m])

    c_xh = pltpu.make_async_copy(x_hbm.at[pl.ds(0, XH), :], x_ref.at[pl.ds(0, XH), :], sem.at[4 * NP])
    c_xr = pltpu.make_async_copy(x_hbm.at[pl.ds(XH, S - XH), :], x_ref.at[pl.ds(XH, S - XH), :],
                                 sem.at[4 * NP + 1])
    c_bq = pltpu.make_async_copy(bqkv_hbm, lbqkv_ref, sem.at[4 * NP + 2])
    c_bo = pltpu.make_async_copy(bwo_hbm, lbwo_ref, sem.at[4 * NP + 3])
    S1 = (NSEG - 3) * SEG
    c_o1 = pltpu.make_async_copy(out_ref.at[pl.ds(0, S1), :], out_hbm.at[pl.ds(0, S1), :], sem.at[4 * NP + 4])
    c_o2 = pltpu.make_async_copy(out_ref.at[pl.ds(S1, S - S1), :], out_hbm.at[pl.ds(S1, S - S1), :],
                                 sem.at[4 * NP + 5])

    def issue(p):
        for m in (1, 2, 3):
            w_copy(m, p).start()

    c_xh.start()
    w_copy(0, 0).start()
    for p in range(DMA_WIN):
        issue(p)
        w_copy(0, p + 1).start()

    r = lax.broadcasted_iota(jnp.int32, (L, 128), 0)
    l = lax.broadcasted_iota(jnp.int32, (L, 128), 1)
    slot = jnp.where(l >= L, l - L, l)
    valid = (l < 2 * L) & ((r < M) | (r >= slot))
    in_h = l < L
    in_g = (l >= L) & (l < 2 * L)
    lo = l < DH - 128
    fill = -1e9 / scale_a
    c_exp = scale_a * LOG2E

    def rows_c(a, c):
        if a.shape[0] == L:
            return a
        return jnp.concatenate([a[M * c:M * c + M], a[2 * M + SEG * c:2 * M + SEG * c + SEG]], axis=0)

    def blk(a, c, pad):
        a = rows_c(a, c)
        a0, a1, a2 = a[:, 0:128], a[:, 128:256], a[:, 256:384]
        z = jnp.zeros((L, 128), F32)
        top = jnp.concatenate([a0, jnp.where(lo, a1, 0.0), z], axis=1)
        bot = jnp.concatenate([z, jnp.where(lo, 0.0, a1), a2], axis=1)
        parts = [top, bot] + ([jnp.zeros((128 - 2 * L, PW), F32)] if pad else [])
        return jnp.concatenate(parts, axis=0).astype(BF16)

    def qk(q, k, chains):
        return [_dot(rows_c(q, c), blk(k, c, False), NT) for c in chains]

    def attn_c(s, v, c):
        s = jnp.concatenate([s, jnp.full((L, 128 - 2 * L), fill, F32)], axis=1)
        s = jnp.where(valid, s, fill)
        mh = jnp.max(jnp.where(in_h, s, -jnp.inf), axis=-1, keepdims=True)
        mg = jnp.max(jnp.where(in_g, s, -jnp.inf), axis=-1, keepdims=True)
        e = jnp.exp2((s - jnp.where(in_h, mh, mg)) * c_exp)
        e = jnp.where(l < 2 * L, e, 0.0)
        ih = _rcp(jnp.sum(jnp.where(in_h, e, 0.0), axis=-1, keepdims=True))
        ig = _rcp(jnp.sum(jnp.where(in_g, e, 0.0), axis=-1, keepdims=True))
        o = _dot(e, blk(v, c, True))
        return jnp.concatenate(
            [o[:, 0:128] * ih, o[:, 128:256] * jnp.where(lo, ih, ig), o[:, 256:384] * ig], axis=1)

    def pv(ss, v, chains):
        os_ = [attn_c(s, v, c) for s, c in zip(ss, chains)]
        if len(chains) == 2:
            return jnp.concatenate([os_[0][0:M], os_[1][0:M], os_[0][M:L], os_[1][M:L]], axis=0)
        return os_[0]

    def seg_rows(s):
        if isinstance(s, int):
            return pl.ds(s * SEG, SEG)
        return pl.ds(pl.multiple_of(s * SEG, SEG), SEG)

    mem0 = mem0_ref[...].astype(F32)
    y_ref[...] = jnp.zeros(y_ref.shape, F32)
    x2_ref[...] = jnp.zeros(x2_ref.shape, F32)
    kb_ref[...] = jnp.zeros(kb_ref.shape, F32)
    vb_ref[...] = jnp.zeros(vb_ref.shape, F32)
    acc0_ref[...] = jnp.zeros(acc0_ref.shape, F32)
    for r_ in (qp_ref, kp_ref, vp_ref):
        r_[0, 0:L, :] = jnp.zeros((L, PW), F32)
    wo_ref[0] = jnp.zeros(wo_ref.shape[1:], U32)
    c_xh.wait()
    h0_ref[0:M, :] = mem0
    h0_ref[M:L, :] = _ln(x_ref[0:SEG, :].astype(F32)).astype(BF16).astype(F32)
    h0_ref[L:L + NPRE * SEG, :] = _ln(x_ref[2 * SEG:(2 + NPRE) * SEG, :].astype(F32)).astype(BF16).astype(F32)
    w_copy(0, 0).wait()
    wk_ref[0] = _pack(lk_ref[0:PW, :].T)

    def startup_body(p, carry):
        for m in (1, 2, 3):
            w_copy(m, p).wait()

        @pl.when(p + 1 < NP)
        def _():
            w_copy(0, p + 1).wait()

        @pl.when(p + DMA_WIN < NP)
        def _():
            issue(p + DMA_WIN)

        @pl.when(p + DMA_WIN + 1 < NP)
        def _():
            w_copy(0, p + DMA_WIN + 1).start()

        @pl.when(p + DMA_WIN == NP)
        def _():
            c_bq.start()
            c_bo.start()
            c_xr.start()

        rows = pl.ds(pl.multiple_of(p * PW, PW), PW)
        pp = jnp.maximum(p - 1, 0)
        ss = qk(qp_ref[pp, 0:L, :], kp_ref[pp, 0:L, :], (0,))
        vprev = vp_ref[pp, 0:L, :]
        woprev = _unpack(wo_ref[pp])
        h = h0_ref[...]
        k = _dot(h, _unpack(wk_ref[p]))
        wq = lq_ref[rows, :].T
        wq_ref[p] = _pack(wq)
        q = _dot(h, wq)
        o = pv(ss, vprev, (0,))
        wv = lv_ref[rows, :].T
        wv_ref[p] = _pack(wv)
        v = _dot(h, wv)
        acc0_ref[...] += _dot(o, woprev)
        wo_ref[p] = _pack(lo_ref[rows, :])
        pn = jnp.minimum(p + 1, NP - 1)
        wk_ref[pn] = _pack(lk_ref[pl.ds(pl.multiple_of(pn * PW, PW), PW), :].T)
        kp_ref[p] = k
        qp_ref[p] = q
        vp_ref[p] = v
        return carry

    lax.fori_loop(0, NP, startup_body, 0)
    o_last = pv(qk(qp_ref[NP - 1, 0:L, :], kp_ref[NP - 1, 0:L, :], (0,)), vp_ref[NP - 1, 0:L, :], (0,))
    acc0 = acc0_ref[...] + _dot(o_last, _unpack(wo_ref[NP - 1]))
    h_ref[0:2 * M, :] = jnp.concatenate([acc0[0:M], mem0], axis=0).astype(BF16)
    h_ref[2 * M:2 * M + SEG, :] = _ln(x_ref[seg_rows(1), :].astype(F32)).astype(BF16)
    h_ref[2 * M + SEG:2 * L, :] = jnp.zeros((SEG, D), BF16)
    y_ref[0:SEG, :] = x_ref[seg_rows(0), :].astype(F32) + acc0[M:L]

    def b_perm_in(j):
        for c in range(NTB):
            if j < 3:
                t_ = lbqkv_ref[c * 128:(c + 1) * 128, j * D:(j + 1) * D].T
            else:
                t_ = lbwo_ref[:, c * 128:(c + 1) * 128]
            tf_ref[j, c] = t_.astype(F32)

    def b_perm_out(j):
        for c in range(NTB):
            t_ = jnp.concatenate([tf_ref[j, c, pl.ds(d, HB, stride=DHB), :] for d in range(DHB)], axis=0)
            t_ = t_.astype(BF16)
            if j < 3:
                bqkvp_ref[c * 64:(c + 1) * 64, j * D:(j + 1) * D] = _pack(t_.T)
            else:
                bwop_ref[:, c * 128:(c + 1) * 128] = _pack(t_)

    rowi = lax.broadcasted_iota(jnp.int32, (HIST, 128), 0)
    fill_b = -1e9 / scale_b
    c_expb = scale_b * LOG2E

    def b_front(lyrs=(0, 1)):
        r0, r1 = SEG * lyrs[0], SEG * lyrs[-1] + SEG
        qkv = _dot(_ln(y_ref[r0:r1, :]).astype(BF16), _unpack(bqkvp_ref[...]))
        for j, dst in ((1, kb_ref), (2, vb_ref)):
            for lyr in lyrs:
                for c in range(NTB):
                    dst[lyr, c, HIST:HIST + SEG, :] = qkv[SEG * lyr - r0:SEG * lyr - r0 + SEG,
                                                          j * D + 128 * c:j * D + 128 * c + 128]
        return qkv[:, 0:D]

    def b_attn(q, t, lyr):
        seg = t - 1 - 2 * lyr
        if q.shape[0] != SEG:
            q = q[SEG * lyr:SEG * lyr + SEG]
        logits = []
        for w in range(W):
            tt = None
            for j in range(NTB):
                pr = q[:, 128 * j:128 * j + 128] * kb_ref[lyr, j, HIST - DIL * w:HIST + SEG - DIL * w, :]
                tt = pr if tt is None else tt + pr
            tt = tt + pltpu.roll(tt, 2 * HB, 1)
            tt = tt + pltpu.roll(tt, HB, 1)
            if w > 0:
                top = jnp.where(rowi >= DIL * w - seg * SEG, tt[0:HIST], fill_b)
                tt = jnp.concatenate([top, tt[HIST:SEG]], axis=0)
            logits.append(tt)
        mx = functools.reduce(jnp.maximum, logits)
        es = [jnp.exp2((t_ - mx) * c_expb) for t_ in logits]
        inv = _rcp(functools.reduce(lambda a, b: a + b, es))
        outs = []
        for j in range(NTB):
            o = None
            for w in range(W):
                c = es[w] * vb_ref[lyr, j, HIST - DIL * w:HIST + SEG - DIL * w, :]
                o = c if o is None else o + c
            outs.append(o * inv)
        for j in range(NTB):
            kb_ref[lyr, j, 0:HIST, :] = kb_ref[lyr, j, SEG:SEG + HIST, :]
            vb_ref[lyr, j, 0:HIST, :] = vb_ref[lyr, j, SEG:SEG + HIST, :]
        return jnp.concatenate(outs, axis=1)

    def b_back(o, lyr):
        return y_ref[SEG * lyr:SEG * lyr + SEG, :] + _dot(o, _unpack(bwop_ref[...]))

    def step(t, chains, pre=False, hook=None, p_b0=P_B0):
        dual = len(chains) == 2
        if pre:
            h = jnp.concatenate([h_ref[0:2 * M, :], h_ref[2 * M + SEG:2 * L, :]], axis=0)
        elif dual:
            h = h_ref[...]
        else:
            h = rows_c(h_ref[...].astype(F32), chains[0])
        x2_res = x2_ref[...] if 1 in chains else None
        st = {}

        def b0():
            z = b_back(b_attn(st["q"], t, 0), 0)
            x2_ref[...] = z
            h_ref[2 * M + SEG:2 * L, :] = _ln(z).astype(BF16)

        def b1():
            z = b_back(b_attn(st["q"], t, 1), 1)
            out_ref[seg_rows(jnp.maximum(t - 3, 0)), :] = z.astype(out_ref.dtype)

        def prj(w_ref, p_ref, p, cols=slice(None)):
            res = _dot(h, _unpack(w_ref[p, :, cols]))
            if pre:
                xs = p_ref[p, pl.ds(pl.multiple_of(L + (t - 2) * SEG, 8), SEG), cols]
                res = jnp.concatenate([res[0:2 * M], xs, res[2 * M:L + M]], axis=0)
            return res

        def opj(o, p):
            return _dot(o.astype(BF16) if dual else o, _unpack(wo_ref[p]))

        k = prj(wk_ref, kp_ref, 0)
        q = prj(wq_ref, qp_ref, 0)
        v = prj(wv_ref, vp_ref, 0)
        acc = None
        o = None
        for p in range(NP):
            ss = qk(q, k, chains)
            if hook is not None:
                hook(p, st)
            elif p == P_BFRONT:
                st["q"] = b_front()
            if p == P_LNX and 0 in chains:
                tn = min(t + 1, NSEG - 1) if isinstance(t, int) else jnp.minimum(t + 1, NSEG - 1)
                h_ref[2 * M:2 * M + SEG, :] = _ln(x_ref[seg_rows(tn), :].astype(F32)).astype(BF16)
            if p + 1 < NP:
                q = prj(wq_ref, qp_ref, p + 1)
                k = prj(wk_ref, kp_ref, p + 1)
            else:
                v = jnp.concatenate([v, prj(wv_ref, vp_ref, p, slice(256, PW))], axis=1)
                acc = acc + opj(o, p - 1)
            o = pv(ss, v, chains)
            if p + 2 < NP:
                v = prj(wv_ref, vp_ref, p + 1)
            elif p + 2 == NP:
                v = prj(wv_ref, vp_ref, p + 1, slice(0, 256))
            elif 1 in chains:
                b1()
            if p != NP - 2:
                d = opj(o, p)
                acc = d if acc is None else acc + d
            if p == p_b0:
                b0()

        if dual:
            h_ref[0:2 * M, :] = acc[0:2 * M].astype(BF16)
            y_ref[0:SEG, :] = x_ref[seg_rows(t), :].astype(F32) + acc[2 * M:2 * M + SEG]
            y_ref[SEG:2 * SEG, :] = x2_res + acc[2 * M + SEG:2 * L]
        elif chains[0] == 0:
            h_ref[0:M, :] = acc[0:M].astype(BF16)
            y_ref[0:SEG, :] = x_ref[seg_rows(t), :].astype(F32) + acc[M:L]
        else:
            h_ref[M:2 * M, :] = acc[0:M].astype(BF16)
            y_ref[SEG:2 * SEG, :] = x2_res + acc[M:L]

    def run(lo_, hi_, chains, pre=False):
        def body(t, carry):
            step(t, chains, pre)
            return carry
        lax.fori_loop(lo_, hi_, body, 0)

    def hook1(p, st):
        if p == P1_PERM:
            c_bq.wait()
            c_bo.wait()
        if P1_PERM <= p < P1_PERM + 4:
            b_perm_in(p - P1_PERM)
        if P1_PERM + 1 <= p < P1_PERM + 5:
            b_perm_out(p - P1_PERM - 1)
        if p == P1_BFRONT:
            st["q"] = b_front((0,))

    step(1, (0,), hook=hook1, p_b0=P1_B0)
    c_xr.wait()
    run(2, 2 + NPRE, (0, 1), pre=True)
    run(2 + NPRE, NSEG, (0, 1))
    c_o1.start()
    run(NSEG, NSEG + 2, (1,))
    z = b_back(b_attn(b_front((1,)), NSEG + 2, 1), 1)
    out_ref[seg_rows(NSEG - 1), :] = z.astype(out_ref.dtype)
    c_o2.start()
    c_o1.wait()
    c_o2.wait()


@functools.partial(jax.jit, static_argnames=("A_seg_len",))
def pallas_interleave_layers__memory_aug_recurrent_mem_tr__sliding_local_dilated__prompt_kernel(
    A_x: jax.Array,
    A_mem0: jax.Array,
    A_Wq: jax.Array,
    A_Wk: jax.Array,
    A_Wv: jax.Array,
    A_Wo: jax.Array,
    A_seg_len: int,
    B_x: jax.Array,
    B_wqkv: jax.Array,
    B_wo: jax.Array,
):
    del B_x
    B, S, D = A_x.shape
    _, H, DH = A_Wq.shape
    M = A_mem0.shape[1]
    SEG = int(A_seg_len)
    assert B == 1 and M == 8 and SEG == 32 and DH == 192 and D == 640 and S % SEG == 0
    NP, PW = H // 2, 2 * DH
    R0 = M + SEG + NPRE * SEG

    x = A_x.reshape(S, D)
    mem0 = A_mem0.reshape(M, D)
    wq = A_Wq.transpose(1, 2, 0).reshape(H * DH, D)
    wk = A_Wk.transpose(1, 2, 0).reshape(H * DH, D)
    wv = A_Wv.transpose(1, 2, 0).reshape(H * DH, D)
    wo = A_Wo.reshape(H * DH, D)

    kern = functools.partial(_kernel, S=S, D=D, H=H, DH=DH, M=M, SEG=SEG, HB=32, W=8, DIL=2)
    hbm = pl.BlockSpec(memory_space=pl.ANY)
    out = pl.pallas_call(
        kern,
        out_shape=jax.ShapeDtypeStruct((S, D), A_x.dtype),
        in_specs=[hbm, pl.BlockSpec(memory_space=pltpu.VMEM), hbm, hbm, hbm, hbm, hbm, hbm],
        out_specs=hbm,
        scratch_shapes=[
            pltpu.VMEM((S, D), BF16),
            pltpu.VMEM((S, D), A_x.dtype),
            pltpu.VMEM((H * DH, D), BF16),
            pltpu.VMEM((H * DH, D), BF16),
            pltpu.VMEM((H * DH, D), BF16),
            pltpu.VMEM((H * DH, D), BF16),
            pltpu.VMEM((NP, D // 2, PW), U32),
            pltpu.VMEM((NP, D // 2, PW), U32),
            pltpu.VMEM((NP, D // 2, PW), U32),
            pltpu.VMEM((NP, PW // 2, D), U32),
            pltpu.VMEM((D, 3 * D), BF16),
            pltpu.VMEM((D, D), BF16),
            pltpu.VMEM((4, D // 128, D, 128), F32),
            pltpu.VMEM((D // 2, 3 * D), U32),
            pltpu.VMEM((D // 2, D), U32),
            pltpu.VMEM((2 * (M + SEG), D), BF16),
            pltpu.VMEM((2 * SEG, D), F32),
            pltpu.VMEM((SEG, D), F32),
            pltpu.VMEM((2, D // 128, 48, 128), F32),
            pltpu.VMEM((2, D // 128, 48, 128), F32),
            pltpu.VMEM((R0, D), F32),
            pltpu.VMEM((M + SEG, D), F32),
            pltpu.VMEM((NP, R0, PW), F32),
            pltpu.VMEM((NP, R0, PW), F32),
            pltpu.VMEM((NP, R0, PW), F32),
            pltpu.SemaphoreType.DMA((4 * NP + 6,)),
        ],
        compiler_params=pltpu.CompilerParams(vmem_limit_bytes=110 * 1024 * 1024),
    )(x, mem0, wq, wk, wv, wo, B_wqkv, B_wo)
    return out.reshape(B, S, D)
```

```python
import functools

import jax
import jax.numpy as jnp
from jax import lax
import jax.experimental.pallas as pl
import jax.experimental.pallas.tpu as pltpu

F32 = jnp.float32
BF16 = jnp.bfloat16
U32 = jnp.uint32
NT = (((1,), (1,)), ((), ()))
NN = (((1,), (0,)), ((), ()))
LOG2E = 1.4426950408889634

NPRE = 8
DMA_WIN = 4
P_BFRONT, P_LNX, P_B0 = 0, 9, 10
P1_PERM, P1_BFRONT, P1_B0 = 2, 10, 14


def _ln(x):
    m = jnp.mean(x, axis=-1, keepdims=True)
    xc = x - m
    v = jnp.mean(xc * xc, axis=-1, keepdims=True)
    return xc * lax.rsqrt(v + 1e-5)


def _dot(a, b, dims=NN):
    return lax.dot_general(a, b, dims, preferred_element_type=F32)


def _rcp(x):
    r = pl.reciprocal(x, approx=True)
    return r * (2.0 - x * r)


def _pack(x):
    return pltpu.bitcast(x, U32)


def _unpack(x):
    return pltpu.bitcast(x, BF16)


def _kernel(x_hbm, mem0_ref, wq_hbm, wk_hbm, wv_hbm, wo_hbm, bqkv_hbm, bwo_hbm,
            out_hbm,
            x_ref, out_ref, lq_ref, lk_ref, lv_ref, lo_ref, wq_ref, wk_ref, wv_ref, wo_ref,
            lbqkv_ref, lbwo_ref, tf_ref, bqkvp_ref, bwop_ref,
            h_ref, y_ref, x2_ref, kb_ref, vb_ref, h0_ref, acc0_ref, q0_ref, k0_ref, v0_ref,
            qp_ref, kp_ref, vp_ref, sem,
            *, S, D, H, DH, M, SEG, HB, W, DIL):
    NSEG = S // SEG
    NP = H // 2
    PW = 2 * DH
    L = M + SEG
    scale_a = DH ** -0.5
    DHB = D // HB
    scale_b = DHB ** -0.5
    NTB = D // 128
    HIST = DIL * W
    R0 = L + NPRE * SEG
    XH = (NPRE + 4) * SEG

    def w_copy(m, p):
        src, dst = ((wk_hbm, lk_ref), (wq_hbm, lq_ref), (wv_hbm, lv_ref), (wo_hbm, lo_ref))[m]
        rows = pl.ds(pl.multiple_of(p * PW, PW), PW)
        return pltpu.make_async_copy(src.at[rows, :], dst.at[rows, :], sem.at[4 * p + m])

    c_xh = pltpu.make_async_copy(x_hbm.at[pl.ds(0, XH), :], x_ref.at[pl.ds(0, XH), :], sem.at[4 * NP])
    c_xr = pltpu.make_async_copy(x_hbm.at[pl.ds(XH, S - XH), :], x_ref.at[pl.ds(XH, S - XH), :],
                                 sem.at[4 * NP + 1])
    c_bq = pltpu.make_async_copy(bqkv_hbm, lbqkv_ref, sem.at[4 * NP + 2])
    c_bo = pltpu.make_async_copy(bwo_hbm, lbwo_ref, sem.at[4 * NP + 3])
    S1 = (NSEG - 3) * SEG
    c_o1 = pltpu.make_async_copy(out_ref.at[pl.ds(0, S1), :], out_hbm.at[pl.ds(0, S1), :], sem.at[4 * NP + 4])
    c_o2 = pltpu.make_async_copy(out_ref.at[pl.ds(S1, S - S1), :], out_hbm.at[pl.ds(S1, S - S1), :],
                                 sem.at[4 * NP + 5])

    def issue(p):
        for m in (1, 2, 3):
            w_copy(m, p).start()

    c_xh.start()
    w_copy(0, 0).start()
    for p in range(DMA_WIN):
        issue(p)
        w_copy(0, p + 1).start()

    r = lax.broadcasted_iota(jnp.int32, (L, 128), 0)
    l = lax.broadcasted_iota(jnp.int32, (L, 128), 1)
    slot = jnp.where(l >= L, l - L, l)
    valid = (l < 2 * L) & ((r < M) | (r >= slot))
    in_h = l < L
    in_g = (l >= L) & (l < 2 * L)
    lo = l < DH - 128
    fill = -1e9 / scale_a
    c_exp = scale_a * LOG2E

    def rows_c(a, c):
        if a.shape[0] == L:
            return a
        return jnp.concatenate([a[M * c:M * c + M], a[2 * M + SEG * c:2 * M + SEG * c + SEG]], axis=0)

    def blk(a, c, pad):
        a = rows_c(a, c)
        a0, a1, a2 = a[:, 0:128], a[:, 128:256], a[:, 256:384]
        z = jnp.zeros((L, 128), F32)
        top = jnp.concatenate([a0, jnp.where(lo, a1, 0.0), z], axis=1)
        bot = jnp.concatenate([z, jnp.where(lo, 0.0, a1), a2], axis=1)
        parts = [top, bot] + ([jnp.zeros((128 - 2 * L, PW), F32)] if pad else [])
        return jnp.concatenate(parts, axis=0).astype(BF16)

    def qk(q, k, chains):
        return [_dot(rows_c(q, c), blk(k, c, False), NT) for c in chains]

    def attn_c(s, v, c):
        s = jnp.concatenate([s, jnp.full((L, 128 - 2 * L), fill, F32)], axis=1)
        s = jnp.where(valid, s, fill)
        mh = jnp.max(jnp.where(in_h, s, -jnp.inf), axis=-1, keepdims=True)
        mg = jnp.max(jnp.where(in_g, s, -jnp.inf), axis=-1, keepdims=True)
        e = jnp.exp2((s - jnp.where(in_h, mh, mg)) * c_exp)
        e = jnp.where(l < 2 * L, e, 0.0)
        ih = _rcp(jnp.sum(jnp.where(in_h, e, 0.0), axis=-1, keepdims=True))
        ig = _rcp(jnp.sum(jnp.where(in_g, e, 0.0), axis=-1, keepdims=True))
        o = _dot(e, blk(v, c, True))
        return jnp.concatenate(
            [o[:, 0:128] * ih, o[:, 128:256] * jnp.where(lo, ih, ig), o[:, 256:384] * ig], axis=1)

    def pv(ss, v, chains):
        os_ = [attn_c(s, v, c) for s, c in zip(ss, chains)]
        if len(chains) == 2:
            return jnp.concatenate([os_[0][0:M], os_[1][0:M], os_[0][M:L], os_[1][M:L]], axis=0)
        return os_[0]

    def seg_rows(s):
        if isinstance(s, int):
            return pl.ds(s * SEG, SEG)
        return pl.ds(pl.multiple_of(s * SEG, SEG), SEG)

    mem0 = mem0_ref[...].astype(F32)
    y_ref[...] = jnp.zeros(y_ref.shape, F32)
    x2_ref[...] = jnp.zeros(x2_ref.shape, F32)
    kb_ref[...] = jnp.zeros(kb_ref.shape, F32)
    vb_ref[...] = jnp.zeros(vb_ref.shape, F32)
    acc0_ref[...] = jnp.zeros(acc0_ref.shape, F32)
    for r_ in (q0_ref, k0_ref, v0_ref):
        r_[0] = jnp.zeros((L, PW), F32)
    wo_ref[0] = jnp.zeros(wo_ref.shape[1:], U32)
    c_xh.wait()
    h0_ref[0:M, :] = mem0
    h0_ref[M:L, :] = _ln(x_ref[0:SEG, :].astype(F32)).astype(BF16).astype(F32)
    h0_ref[L:L + NPRE * SEG, :] = _ln(x_ref[2 * SEG:(2 + NPRE) * SEG, :].astype(F32)).astype(BF16).astype(F32)
    w_copy(0, 0).wait()
    wk_ref[0] = _pack(lk_ref[0:PW, :].T)

    def startup_body(p, carry):
        for m in (1, 2, 3):
            w_copy(m, p).wait()

        @pl.when(p + 1 < NP)
        def _():
            w_copy(0, p + 1).wait()

        @pl.when(p + DMA_WIN < NP)
        def _():
            issue(p + DMA_WIN)

        @pl.when(p + DMA_WIN + 1 < NP)
        def _():
            w_copy(0, p + DMA_WIN + 1).start()

        @pl.when(p + DMA_WIN == NP)
        def _():
            c_bq.start()
            c_bo.start()
            c_xr.start()

        rows = pl.ds(pl.multiple_of(p * PW, PW), PW)
        pp = jnp.maximum(p - 1, 0)
        ss = qk(q0_ref[pp], k0_ref[pp], (0,))
        vprev = v0_ref[pp]
        woprev = _unpack(wo_ref[pp])
        h = h0_ref[...]
        k = _dot(h, _unpack(wk_ref[p]))
        wq = lq_ref[rows, :].T
        wq_ref[p] = _pack(wq)
        q = _dot(h, wq)
        o = pv(ss, vprev, (0,))
        wv = lv_ref[rows, :].T
        wv_ref[p] = _pack(wv)
        v = _dot(h, wv)
        acc0_ref[...] += _dot(o, woprev)
        wo_ref[p] = _pack(lo_ref[rows, :])
        pn = jnp.minimum(p + 1, NP - 1)
        wk_ref[pn] = _pack(lk_ref[pl.ds(pl.multiple_of(pn * PW, PW), PW), :].T)
        for val, r0_, rp_ in ((k, k0_ref, kp_ref), (q, q0_ref, qp_ref), (v, v0_ref, vp_ref)):
            r0_[p] = val[0:L]
            rp_[p] = _pack(val[L:R0].astype(BF16))
        return carry

    lax.fori_loop(0, NP, startup_body, 0)
    o_last = pv(qk(q0_ref[NP - 1], k0_ref[NP - 1], (0,)), v0_ref[NP - 1], (0,))
    acc0 = acc0_ref[...] + _dot(o_last, _unpack(wo_ref[NP - 1]))
    h_ref[0:2 * M, :] = jnp.concatenate([acc0[0:M], mem0], axis=0).astype(BF16)
    h_ref[2 * M:2 * M + SEG, :] = _ln(x_ref[seg_rows(1), :].astype(F32)).astype(BF16)
    h_ref[2 * M + SEG:2 * L, :] = jnp.zeros((SEG, D), BF16)
    y_ref[0:SEG, :] = x_ref[seg_rows(0), :].astype(F32) + acc0[M:L]

    def b_perm_in(j):
        for c in range(NTB):
            if j < 3:
                t_ = lbqkv_ref[c * 128:(c + 1) * 128, j * D:(j + 1) * D].T
            else:
                t_ = lbwo_ref[:, c * 128:(c + 1) * 128]
            tf_ref[j, c] = t_.astype(F32)

    def b_perm_out(j):
        for c in range(NTB):
            t_ = jnp.concatenate([tf_ref[j, c, pl.ds(d, HB, stride=DHB), :] for d in range(DHB)], axis=0)
            t_ = t_.astype(BF16)
            if j < 3:
                bqkvp_ref[c * 64:(c + 1) * 64, j * D:(j + 1) * D] = _pack(t_.T)
            else:
                bwop_ref[:, c * 128:(c + 1) * 128] = _pack(t_)

    rowi = lax.broadcasted_iota(jnp.int32, (HIST, 128), 0)
    fill_b = -1e9 / scale_b
    c_expb = scale_b * LOG2E

    def b_front(lyrs=(0, 1)):
        r0, r1 = SEG * lyrs[0], SEG * lyrs[-1] + SEG
        qkv = _dot(_ln(y_ref[r0:r1, :]).astype(BF16), _unpack(bqkvp_ref[...]))
        for j, dst in ((1, kb_ref), (2, vb_ref)):
            for lyr in lyrs:
                for c in range(NTB):
                    dst[lyr, c, HIST:HIST + SEG, :] = qkv[SEG * lyr - r0:SEG * lyr - r0 + SEG,
                                                          j * D + 128 * c:j * D + 128 * c + 128]
        return qkv[:, 0:D]

    def b_attn(q, t, lyr):
        seg = t - 1 - 2 * lyr
        if q.shape[0] != SEG:
            q = q[SEG * lyr:SEG * lyr + SEG]
        logits = []
        for w in range(W):
            tt = None
            for j in range(NTB):
                pr = q[:, 128 * j:128 * j + 128] * kb_ref[lyr, j, HIST - DIL * w:HIST + SEG - DIL * w, :]
                tt = pr if tt is None else tt + pr
            tt = tt + pltpu.roll(tt, 2 * HB, 1)
            tt = tt + pltpu.roll(tt, HB, 1)
            if w > 0:
                top = jnp.where(rowi >= DIL * w - seg * SEG, tt[0:HIST], fill_b)
                tt = jnp.concatenate([top, tt[HIST:SEG]], axis=0)
            logits.append(tt)
        mx = functools.reduce(jnp.maximum, logits)
        es = [jnp.exp2((t_ - mx) * c_expb) for t_ in logits]
        inv = _rcp(functools.reduce(lambda a, b: a + b, es))
        outs = []
        for j in range(NTB):
            o = None
            for w in range(W):
                c = es[w] * vb_ref[lyr, j, HIST - DIL * w:HIST + SEG - DIL * w, :]
                o = c if o is None else o + c
            outs.append(o * inv)
        for j in range(NTB):
            kb_ref[lyr, j, 0:HIST, :] = kb_ref[lyr, j, SEG:SEG + HIST, :]
            vb_ref[lyr, j, 0:HIST, :] = vb_ref[lyr, j, SEG:SEG + HIST, :]
        return jnp.concatenate(outs, axis=1)

    def b_back(o, lyr):
        return y_ref[SEG * lyr:SEG * lyr + SEG, :] + _dot(o, _unpack(bwop_ref[...]))

    def step(t, chains, pre=False, hook=None, p_b0=P_B0):
        dual = len(chains) == 2
        if pre:
            h = jnp.concatenate([h_ref[0:2 * M, :], h_ref[2 * M + SEG:2 * L, :]], axis=0)
        elif dual:
            h = h_ref[...]
        else:
            h = rows_c(h_ref[...].astype(F32), chains[0])
        x2_res = x2_ref[...] if 1 in chains else None
        st = {}

        def b0():
            z = b_back(b_attn(st["q"], t, 0), 0)
            x2_ref[...] = z
            h_ref[2 * M + SEG:2 * L, :] = _ln(z).astype(BF16)

        def b1():
            z = b_back(b_attn(st["q"], t, 1), 1)
            out_ref[seg_rows(jnp.maximum(t - 3, 0)), :] = z.astype(out_ref.dtype)

        def prj(w_ref, p_ref, p, cols=slice(None)):
            res = _dot(h, _unpack(w_ref[p, :, cols]))
            if pre:
                xs = _unpack(p_ref[p, pl.ds(pl.multiple_of((t - 2) * (SEG // 2), SEG // 2), SEG // 2), cols]).astype(F32)
                res = jnp.concatenate([res[0:2 * M], xs, res[2 * M:L + M]], axis=0)
            return res

        def opj(o, p):
            return _dot(o.astype(BF16) if dual else o, _unpack(wo_ref[p]))

        k = prj(wk_ref, kp_ref, 0)
        q = prj(wq_ref, qp_ref, 0)
        v = prj(wv_ref, vp_ref, 0)
        acc = None
        o = None
        for p in range(NP):
            ss = qk(q, k, chains)
            if hook is not None:
                hook(p, st)
            elif p == P_BFRONT:
                st["q"] = b_front()
            if p == P_LNX and 0 in chains:
                tn = min(t + 1, NSEG - 1) if isinstance(t, int) else jnp.minimum(t + 1, NSEG - 1)
                h_ref[2 * M:2 * M + SEG, :] = _ln(x_ref[seg_rows(tn), :].astype(F32)).astype(BF16)
            if p + 1 < NP:
                q = prj(wq_ref, qp_ref, p + 1)
                k = prj(wk_ref, kp_ref, p + 1)
            else:
                v = jnp.concatenate([v, prj(wv_ref, vp_ref, p, slice(256, PW))], axis=1)
                acc = acc + opj(o, p - 1)
            o = pv(ss, v, chains)
            if p + 2 < NP:
                v = prj(wv_ref, vp_ref, p + 1)
            elif p + 2 == NP:
                v = prj(wv_ref, vp_ref, p + 1, slice(0, 256))
            elif 1 in chains:
                b1()
            if p != NP - 2:
                d = opj(o, p)
                acc = d if acc is None else acc + d
            if p == p_b0:
                b0()

        if dual:
            h_ref[0:2 * M, :] = acc[0:2 * M].astype(BF16)
            y_ref[0:SEG, :] = x_ref[seg_rows(t), :].astype(F32) + acc[2 * M:2 * M + SEG]
            y_ref[SEG:2 * SEG, :] = x2_res + acc[2 * M + SEG:2 * L]
        elif chains[0] == 0:
            h_ref[0:M, :] = acc[0:M].astype(BF16)
            y_ref[0:SEG, :] = x_ref[seg_rows(t), :].astype(F32) + acc[M:L]
        else:
            h_ref[M:2 * M, :] = acc[0:M].astype(BF16)
            y_ref[SEG:2 * SEG, :] = x2_res + acc[M:L]

    def run(lo_, hi_, chains, pre=False):
        def body(t, carry):
            step(t, chains, pre)
            return carry
        lax.fori_loop(lo_, hi_, body, 0)

    def hook1(p, st):
        if p == P1_PERM:
            c_bq.wait()
            c_bo.wait()
        if P1_PERM <= p < P1_PERM + 4:
            b_perm_in(p - P1_PERM)
        if P1_PERM + 1 <= p < P1_PERM + 5:
            b_perm_out(p - P1_PERM - 1)
        if p == P1_BFRONT:
            st["q"] = b_front((0,))

    step(1, (0,), hook=hook1, p_b0=P1_B0)
    c_xr.wait()
    run(2, 2 + NPRE, (0, 1), pre=True)
    run(2 + NPRE, NSEG, (0, 1))
    c_o1.start()
    run(NSEG, NSEG + 2, (1,))
    z = b_back(b_attn(b_front((1,)), NSEG + 2, 1), 1)
    out_ref[seg_rows(NSEG - 1), :] = z.astype(out_ref.dtype)
    c_o2.start()
    c_o1.wait()
    c_o2.wait()


@functools.partial(jax.jit, static_argnames=("A_seg_len",))
def pallas_interleave_layers__memory_aug_recurrent_mem_tr__sliding_local_dilated__prompt_kernel(
    A_x: jax.Array,
    A_mem0: jax.Array,
    A_Wq: jax.Array,
    A_Wk: jax.Array,
    A_Wv: jax.Array,
    A_Wo: jax.Array,
    A_seg_len: int,
    B_x: jax.Array,
    B_wqkv: jax.Array,
    B_wo: jax.Array,
):
    del B_x
    B, S, D = A_x.shape
    _, H, DH = A_Wq.shape
    M = A_mem0.shape[1]
    SEG = int(A_seg_len)
    assert B == 1 and M == 8 and SEG == 32 and DH == 192 and D == 640 and S % SEG == 0
    NP, PW = H // 2, 2 * DH
    R0 = M + SEG + NPRE * SEG

    x = A_x.reshape(S, D)
    mem0 = A_mem0.reshape(M, D)
    wq = A_Wq.transpose(1, 2, 0).reshape(H * DH, D)
    wk = A_Wk.transpose(1, 2, 0).reshape(H * DH, D)
    wv = A_Wv.transpose(1, 2, 0).reshape(H * DH, D)
    wo = A_Wo.reshape(H * DH, D)

    kern = functools.partial(_kernel, S=S, D=D, H=H, DH=DH, M=M, SEG=SEG, HB=32, W=8, DIL=2)
    hbm = pl.BlockSpec(memory_space=pl.ANY)
    out = pl.pallas_call(
        kern,
        out_shape=jax.ShapeDtypeStruct((S, D), A_x.dtype),
        in_specs=[hbm, pl.BlockSpec(memory_space=pltpu.VMEM), hbm, hbm, hbm, hbm, hbm, hbm],
        out_specs=hbm,
        scratch_shapes=[
            pltpu.VMEM((S, D), BF16),
            pltpu.VMEM((S, D), A_x.dtype),
            pltpu.VMEM((H * DH, D), BF16),
            pltpu.VMEM((H * DH, D), BF16),
            pltpu.VMEM((H * DH, D), BF16),
            pltpu.VMEM((H * DH, D), BF16),
            pltpu.VMEM((NP, D // 2, PW), U32),
            pltpu.VMEM((NP, D // 2, PW), U32),
            pltpu.VMEM((NP, D // 2, PW), U32),
            pltpu.VMEM((NP, PW // 2, D), U32),
            pltpu.VMEM((D, 3 * D), BF16),
            pltpu.VMEM((D, D), BF16),
            pltpu.VMEM((4, D // 128, D, 128), F32),
            pltpu.VMEM((D // 2, 3 * D), U32),
            pltpu.VMEM((D // 2, D), U32),
            pltpu.VMEM((2 * (M + SEG), D), BF16),
            pltpu.VMEM((2 * SEG, D), F32),
            pltpu.VMEM((SEG, D), F32),
            pltpu.VMEM((2, D // 128, 48, 128), F32),
            pltpu.VMEM((2, D // 128, 48, 128), F32),
            pltpu.VMEM((R0, D), F32),
            pltpu.VMEM((M + SEG, D), F32),
            pltpu.VMEM((NP, M + SEG, PW), F32),
            pltpu.VMEM((NP, M + SEG, PW), F32),
            pltpu.VMEM((NP, M + SEG, PW), F32),
            pltpu.VMEM((NP, NPRE * SEG // 2, PW), U32),
            pltpu.VMEM((NP, NPRE * SEG // 2, PW), U32),
            pltpu.VMEM((NP, NPRE * SEG // 2, PW), U32),
            pltpu.SemaphoreType.DMA((4 * NP + 6,)),
        ],
        compiler_params=pltpu.CompilerParams(vmem_limit_bytes=110 * 1024 * 1024),
    )(x, mem0, wq, wk, wv, wo, B_wqkv, B_wo)
    return out.reshape(B, S, D)
```
